```python
import jax
import jax.numpy as jnp

def _softmax(x, axis=-1):
    return jax.nn.softmax(x, axis=axis)
def _gelu(x):
    return jax.nn.gelu(x, approximate=True)
def _silu(x):
    return jax.nn.silu(x)
def _sigmoid(x):
    return jax.nn.sigmoid(x)
def _layernorm(x, axis=-1, eps=1e-5):
    m = jnp.mean(x, axis=axis, keepdims=True)
    v = jnp.var(x, axis=axis, keepdims=True)
    return (x - m) / jnp.sqrt(v + eps)
def _scatter_add(tgt, idx, src, axis=0):
    return tgt.at[idx].add(src)
def _segment_sum(src, seg, n):
    return jax.ops.segment_sum(src, seg, n)
class _Rng:
    def __init__(self, key):
        self._k = key
    def _next(self):
        self._k, sub = jax.random.split(self._k)
        return sub
    def normal(self, shape):
        return jax.random.normal(self._next(), shape, dtype=jnp.bfloat16)
    def randint(self, lo, hi, shape):
        return jax.random.randint(self._next(), shape, lo, hi, dtype=jnp.int32)
    def uniform(self, shape, lo=0.0, hi=1.0):
        return jax.random.uniform(self._next(), shape, jnp.bfloat16, lo, hi)
    def permutation(self, n):
        return jax.random.permutation(self._next(), n)


kernel_name = 'parallel_sum__ssm_conv_s5__moe_arch_mod__prompt'

def setup_inputs():
    _rng = _Rng(jax.random.key(int.from_bytes(__import__("os").urandom(4), "little")))
    _w = (lambda a: (lambda t: t.astype(jnp.bfloat16) if jnp.issubdtype(t.dtype, jnp.floating) else t)(jnp.asarray(a)))
    def _A_setup():
        B, S, D = 1, 2048, 1024
        P = D
        Lambda_re = -0.5 * jnp.exp((lambda *s: _rng.normal(s) * 0.05)(P))
        Lambda_im = (lambda *s: _rng.normal(s) * 0.05)(P) * 1.0
        B_re = (lambda *s: _rng.normal(s) * 0.05)(P, D) * (D ** -0.5)
        B_im = (lambda *s: _rng.normal(s) * 0.05)(P, D) * (D ** -0.5)
        C_re = (lambda *s: _rng.normal(s) * 0.05)(D, P) * (P ** -0.5)
        C_im = (lambda *s: _rng.normal(s) * 0.05)(D, P) * (P ** -0.5)
        log_dt = (lambda *s: _rng.normal(s) * 0.05)(P) * 0.3 - 2.0
        Dskip = (lambda *s: _rng.normal(s) * 0.05)(D)
        return {
            "x": _w((lambda *s: _rng.normal(s) * 0.05)(B, S, D)),
            "Lambda_re": _w(Lambda_re),
            "Lambda_im": _w(Lambda_im),
            "B_re": _w(B_re),
            "B_im": _w(B_im),
            "C_re": _w(C_re),
            "C_im": _w(C_im),
            "log_dt": _w(log_dt),
            "Dskip": _w(Dskip),
        }
    _A_in = _A_setup()

    def _B_setup():
        B, S, D, F, C = 1, 2048, 1024, 3584, 2
        return {
            "x": _w((lambda *s: _rng.normal(s) * 0.05)(B, S, D)),
            "w_r": _w((lambda *s: _rng.normal(s) * 0.05)(D)),
            "w_gate": _w((lambda *s: _rng.normal(s) * 0.05)(D, F)),
            "w_up": _w((lambda *s: _rng.normal(s) * 0.05)(D, F)),
            "w_down": _w((lambda *s: _rng.normal(s) * 0.05)(F, D)),
        }
    _B_in = _B_setup()

    return {
        "A_x": _A_in["x"],
        "A_Lambda_re": _A_in["Lambda_re"],
        "A_Lambda_im": _A_in["Lambda_im"],
        "A_B_re": _A_in["B_re"],
        "A_B_im": _A_in["B_im"],
        "A_C_re": _A_in["C_re"],
        "A_C_im": _A_in["C_im"],
        "A_log_dt": _A_in["log_dt"],
        "A_Dskip": _A_in["Dskip"],
        "B_x": _B_in["x"],
        "B_w_r": _B_in["w_r"],
        "B_w_gate": _B_in["w_gate"],
        "B_w_up": _B_in["w_up"],
        "B_w_down": _B_in["w_down"],
    }

def reference(A_x, A_Lambda_re, A_Lambda_im, A_B_re, A_B_im, A_C_re, A_C_im, A_log_dt, A_Dskip, B_x, B_w_r, B_w_gate, B_w_up, B_w_down):
    def _A_ref(x, Lambda_re, Lambda_im, B_re, B_im, C_re, C_im, log_dt, Dskip):
        Bsz, L, H = x.shape
        Lam = Lambda_re + 1j * Lambda_im
        Bmat = B_re + 1j * B_im
        Cmat = C_re + 1j * C_im
        dt = jnp.exp(log_dt)
        Lam_bar = jnp.exp(dt * Lam)
        B_bar = ((Lam_bar - 1.0) / Lam)[:, None] * Bmat
        Bu = jnp.einsum("bld,pd->blp", x + 0j, B_bar)
        h = jnp.zeros_like(Bu[:, 0, :])
        hs = []
        for t in range(L):
            h = Lam_bar[None, :] * h + Bu[:, t, :]
            hs.append(h)
        hseq = jnp.stack(hs, 1)
        y = 2.0 * jnp.einsum("blp,dp->bld", hseq, Cmat).real + x * Dskip[None, None, :]
        return y

    def _B_ref(x, w_r, w_gate, w_up, w_down):
        B, S, D = x.shape
        C = 2
        r = x @ w_r
        idx = jnp.argsort(-r, axis=-1)[:, :C]
        idx_e = jnp.repeat(idx.reshape(B, C, 1), D, axis=2)
        x_sel = jnp.take_along_axis(x, idx_e, axis=1)
        g = _silu(x_sel @ w_gate)
        u = x_sel @ w_up
        y = (g * u) @ w_down
        r_sel = _sigmoid(jnp.take_along_axis(r, idx, axis=1))
        y = y * r_sel.reshape(B, C, 1)
        b_off = (jnp.arange(B) * S).reshape(B, 1)
        flat_idx = (idx + b_off).reshape(B * C)
        zero = (x * 0.0).reshape(B * S, D)
        upd = _scatter_add(zero, flat_idx, y.reshape(B * C, D), axis=0)
        return x + upd.reshape(B, S, D)

    x = A_x
    xn = _layernorm(x, axis=-1)
    return x + _A_ref(xn, A_Lambda_re, A_Lambda_im, A_B_re, A_B_im, A_C_re, A_C_im, A_log_dt, A_Dskip) + _B_ref(xn, B_w_r, B_w_gate, B_w_up, B_w_down)
```

```python
import functools
import jax
import jax.numpy as jnp
from jax import lax
import jax.experimental.pallas as pl
import jax.experimental.pallas.tpu as pltpu

L = 2048
D = 1024
P = 1024
F = 3584
T = 256
N = L // T
TS = 2 * T + 4
TH = T + 4
NT = (((1,), (1,)), ((), ()))
NN = (((1,), (0,)), ((), ()))
f32 = jnp.float32
bf16 = jnp.bfloat16
EPS_BF16 = 1.0013580322265625e-05
B_PIECES = (256, 256, 512, 1024)
NS = 3
LNG = 16
KU = 512


def _rb(v):
    return v.astype(bf16).astype(f32)


def _row(v8):
    return jnp.concatenate([v8[j:j + 1, :] for j in range(8)], axis=1)


def _dot(a, b, dims):
    return lax.dot_general(a, b, dims, preferred_element_type=f32)


def _interleave(main, extra):
    extra = list(extra)
    n = len(main)
    for i, m in enumerate(main):
        m()
        for e in extra[i * len(extra) // n:(i + 1) * len(extra) // n]:
            e()


def _kernel(x_hbm, lre_hbm, lim_hbm, ldt_hbm, dsk_hbm, wr_hbm, bre_hbm, bim_hbm, cre_hbm, cim_hbm,
            wg_hbm, wu_hbm, wd_hbm, out_hbm,
            x_v, xn_v, b_v, cre_v, cim_v, wg_v, wu_v, wd_v, out_v, sm_v, act_v,
            S0, S1, S2, H0, H1, sem_x, sem_b, sem_c, sem_w, sem_o, sem_s, sem_p, sem_f, sem_l):
    S = (S0, S1, S2)
    H = (H0, H1)

    def cp_x(j):
        return pltpu.make_async_copy(x_hbm.at[j * T:(j + 1) * T, :], x_v.at[j * T:(j + 1) * T, :], sem_x.at[j])

    b_off = [0]
    for n in B_PIECES:
        b_off.append(b_off[-1] + n)

    def cp_b(k):
        lo, hi = b_off[k], b_off[k + 1]
        src = bre_hbm if lo < P else bim_hbm
        assert (lo < P) == (hi <= P)
        return pltpu.make_async_copy(src.at[lo % P:lo % P + hi - lo, :], b_v.at[lo:hi, :], sem_b.at[k])

    cp_c = [pltpu.make_async_copy(cre_hbm, cre_v, sem_c.at[0]), pltpu.make_async_copy(cim_hbm, cim_v, sem_c.at[1])]
    cp_w = [pltpu.make_async_copy(wg_hbm, wg_v, sem_w.at[0]), pltpu.make_async_copy(wu_hbm, wu_v, sem_w.at[1]),
            pltpu.make_async_copy(wd_hbm, wd_v, sem_w.at[2])]
    cp_s = [pltpu.make_async_copy(h, sm_v.at[i], sem_s.at[i])
            for i, h in enumerate((lre_hbm, lim_hbm, ldt_hbm, dsk_hbm, wr_hbm))]

    def cp_o(j):
        return pltpu.make_async_copy(out_v.at[j * T:(j + 1) * T, :], out_hbm.at[j * T:(j + 1) * T, :], sem_o.at[j])

    order = ([cp_x(0)] + cp_s + [cp_x(1), cp_b(0), cp_b(1), cp_b(2), cp_x(2), cp_b(3)] + cp_c
             + [cp_x(jj) for jj in range(3, N)] + cp_w)
    for c in order:
        c.start()
        pl.semaphore_signal(sem_f, 1)
        pl.semaphore_wait(sem_f, 1)

    cp_x(0).wait()
    for c in cp_s:
        c.wait()
    dsk1 = _row(sm_v[3].astype(f32)) + 1.0
    wr = _row(sm_v[4].astype(f32))

    tk = {"m1": jnp.full((LNG, 1), -jnp.inf, f32), "m2": jnp.full((LNG, 1), -jnp.inf, f32),
          "i1": jnp.full((LNG, 1), float(L), f32), "i2": jnp.full((LNG, 1), float(L), f32)}
    row_iota = lax.broadcasted_iota(jnp.int32, (LNG, 1), 0).astype(f32)

    def ln(j, chain):
        for g in range(T // LNG):
            r0 = j * T + g * LNG
            x = jnp.concatenate([x_v[r0 + a:r0 + a + 8, :].astype(f32) for a in range(0, LNG, 8)], axis=0)
            mu = jnp.sum(x, axis=-1, keepdims=True) * (1.0 / D)
            if chain:
                mu = mu + jnp.where(tk["m1"] > jnp.inf, 1.0, 0.0)
            mb = _rb(mu)
            xc = x - mb
            ex2 = jnp.sum(xc * xc, axis=-1, keepdims=True) * (1.0 / D)
            dm = mu - mb
            var = jnp.maximum(ex2 - dm * dm, 0.0)
            den = _rb(jnp.sqrt(_rb(_rb(var) + EPS_BF16)))
            xn = xc * (1.0 / den)
            xn_v[r0 // 2:(r0 + LNG) // 2, :] = pltpu.bitcast(xn.astype(bf16), jnp.uint32)
            out_v[r0:r0 + LNG, :] = x + xn * dsk1
            r = _rb(jnp.sum(xn * wr, axis=-1, keepdims=True))
            idx = row_iota + float(r0)
            is1 = r > tk["m1"]
            is2 = r > tk["m2"]
            tk["m2"] = jnp.where(is1, tk["m1"], jnp.where(is2, r, tk["m2"]))
            tk["i2"] = jnp.where(is1, tk["i1"], jnp.where(is2, idx, tk["i2"]))
            tk["m1"] = jnp.where(is1, r, tk["m1"])
            tk["i1"] = jnp.where(is1, idx, tk["i1"])

    def xn_lhs(r0, r1, c0, c1):
        return pltpu.bitcast(xn_v[r0 // 2:r1 // 2, c0:c1], bf16)

    def s_store(j, kk, val):
        S[j % NS][pl.ds((kk % 8) * TS + kk // 8, T, stride=2), :] = val

    def mm1_cols(j, lo, hi, nchunk=1):
        bu = _dot(xn_lhs(j * T, (j + nchunk) * T, 0, D), b_v[lo:hi, :], NT)
        for c in range(nchunk):
            for q in range((hi - lo) // 128):
                s_store(j + c, lo // 128 + q, bu[c * T:(c + 1) * T, q * 128:(q + 1) * 128])

    def mm1_units(j):
        acc = {}

        def unit(q, h):
            def run():
                part = _dot(xn_lhs(j * T, (j + 1) * T, h * KU, (h + 1) * KU),
                            b_v[q * 128:(q + 1) * 128, h * KU:(h + 1) * KU], NT)
                if h == 0:
                    acc[q] = part
                else:
                    s_store(j, q, acc.pop(q) + part)
            return run
        return [unit(q, h) for q in range(16) for h in range(D // KU)]

    def scan(j, hr, hi):
        s = S[j % NS]
        h = H[j % 2]
        for t2 in range(T // 2):
            outs = []
            for t in (2 * t2, 2 * t2 + 1):
                br = s[pl.ds(2 * t, 8, stride=TS), :]
                bi = s[pl.ds(2 * t + 1, 8, stride=TS), :]
                ur = fr * br - fi * bi
                ui = fr * bi + fi * br
                nr_ = ar * hr - ai * hi + ur
                ni_ = ar * hi + ai * hr + ui
                hr, hi = nr_, ni_
                outs.append((hr, hi))
            h[pl.ds(2 * t2, 8, stride=TH), :] = pltpu.pack_elementwise(
                [outs[0][0], outs[1][0]], packed_dtype=bf16)
            h[pl.ds(2 * t2 + 1, 8, stride=TH), :] = pltpu.pack_elementwise(
                [outs[0][1], outs[1][1]], packed_dtype=bf16)
        return hr, hi

    def h_blk(j, k):
        return pltpu.bitcast(H[j % 2][pl.ds((k % 8) * TH + k // 8, T // 2, stride=2), :], bf16)

    def h_lhs(j):
        hre = jnp.concatenate([h_blk(j, k) for k in range(8)], axis=1)
        him = jnp.concatenate([h_blk(j, k) for k in range(8, 16)], axis=1)
        return hre, him

    def mm2(j):
        rows = slice(j * T, (j + 1) * T)
        hre, him = h_lhs(j)
        y = _dot(hre, cre_v[...], NT) - _dot(him, cim_v[...], NT)
        out_v[rows, :] = out_v[rows, :] + y

    def mm2_units(j):
        rows = slice(j * T, (j + 1) * T)
        st2 = {}

        def unit(q, u):
            def run():
                if "h" not in st2:
                    st2["h"] = h_lhs(j)
                hre, him = st2["h"]
                cols = slice(q * 128, (q + 1) * 128)
                ks = slice((u % 2) * KU, (u % 2 + 1) * KU)
                if u < 2:
                    part = _dot(hre[:, ks], cre_v[cols, ks], NT)
                    st2[q] = part if u == 0 else st2[q] + part
                else:
                    part = _dot(him[:, ks], cim_v[cols, ks], NT)
                    if u == 2:
                        st2[q] = st2[q] - part
                    else:
                        out_v[rows, cols] = out_v[rows, cols] + (st2.pop(q) - part)
            return run
        return [unit(q, u) for q in range(8) for u in range(4)]

    st = {}

    def top2():
        vals = jnp.concatenate([tk["m1"], tk["m2"]], axis=0)
        idxs = jnp.concatenate([tk["i1"], tk["i2"]], axis=0)
        m1 = jnp.max(vals, axis=0, keepdims=True)
        i1f = jnp.min(jnp.where(vals == m1, idxs, float(L)), axis=0, keepdims=True)
        vals2 = jnp.where(idxs == i1f, -jnp.inf, vals)
        m2 = jnp.max(vals2, axis=0, keepdims=True)
        i2f = jnp.min(jnp.where(vals2 == m2, idxs, float(L)), axis=0, keepdims=True)
        i1 = jnp.clip(jnp.min(i1f).astype(jnp.int32), 0, L - 1)
        i2 = jnp.clip(jnp.min(i2f).astype(jnp.int32), 0, L - 1)

        def gather(i):
            base = pl.multiple_of((i // 16) * 8, 8)
            tile = pltpu.bitcast(xn_v[pl.ds(base, 8), :], bf16).astype(f32)
            sel = lax.broadcasted_iota(jnp.int32, (16, D), 0) == (i % 16)
            return jnp.sum(jnp.where(sel, tile, 0.0), axis=0, keepdims=True)

        rid = lax.broadcasted_iota(jnp.int32, (16, D), 0)
        st["xs"] = jnp.where(rid == 0, gather(i1), jnp.where(rid == 1, gather(i2), 0.0)).astype(bf16)
        st["i"] = (i1, i2)
        st["m"] = (m1, m2)

    def gu_units():
        def unit(k, w, h):
            def run():
                cols = slice(k * 128, (k + 1) * 128)
                ks = slice(h * KU, (h + 1) * KU)
                part = _dot(st["xs"][:, ks], (wg_v, wu_v)[w][ks, cols], NN)
                key = ("gu", k, w)
                st[key] = part if h == 0 else st[key] + part
                if w == 1 and h == 1:
                    g = st.pop(("gu", k, 0))
                    u = st.pop(("gu", k, 1))
                    act_v[:, cols] = (g * jax.nn.sigmoid(g) * u).astype(bf16)
            return run
        return [unit(k, w, h) for k in range(F // 128) for w in range(2) for h in range(2)]

    def down_units():
        def unit(q, u):
            def run():
                cols = slice(q * 128, (q + 1) * 128)
                ks = slice(u * KU, (u + 1) * KU)
                part = _dot(act_v[:, ks], wd_v[ks, cols], NN)
                key = ("y", q)
                st[key] = part if u == 0 else st[key] + part
            return run
        return [unit(q, u) for q in range(8) for u in range(F // KU)]

    def patch(nsent):
        i1, i2 = st["i"]
        m1, m2 = st["m"]
        y = jnp.concatenate([st[("y", q)] for q in range(8)], axis=1)
        rid = lax.broadcasted_iota(jnp.int32, (16, D), 0)
        rs = jnp.where(rid == 0, m1, m2)
        y = y * jax.nn.sigmoid(rs)
        gs = []
        for k, i in enumerate((i1, i2)):
            g0 = pl.multiple_of((i // 8) * 8, 8)
            sel = lax.broadcasted_iota(jnp.int32, (8, D), 0) == (i - g0)
            blk = out_v[pl.ds(g0, 8), :]
            out_v[pl.ds(g0, 8), :] = blk + jnp.where(sel, y[k:k + 1, :], 0.0)
            gs.append(g0)
        c1 = pltpu.make_async_copy(out_v.at[pl.ds(gs[0], 8), :], out_hbm.at[pl.ds(gs[0], 8), :], sem_p.at[0])
        c2 = pltpu.make_async_copy(out_v.at[pl.ds(gs[1], 8), :], out_hbm.at[pl.ds(gs[1], 8), :], sem_p.at[1])
        p1 = gs[0] < nsent * T
        p2 = jnp.logical_and(gs[1] < nsent * T, gs[1] != gs[0])

        @pl.when(p1)
        def _():
            c1.start()

        @pl.when(p2)
        def _():
            c2.start()

        def finish():
            @pl.when(p1)
            def _():
                c1.wait()

            @pl.when(p2)
            def _():
                c2.wait()
        return finish

    ln(0, False)
    cp_x(1).wait()
    ln(1, False)
    cp_b(0).wait()
    mm1_cols(0, b_off[0], b_off[1], 2)
    lre = sm_v[0].astype(f32)
    lim = sm_v[1].astype(f32)
    dt = _rb(jnp.exp(sm_v[2].astype(f32)))
    mag = jnp.exp(dt * lre)
    ang = dt * lim
    ar = mag * jnp.cos(ang)
    ai = mag * jnp.sin(ang)
    nr = ar - 1.0
    inv = 2.0 / (lre * lre + lim * lim)
    fr = (nr * lre + ai * lim) * inv
    fi = (ai * lre - nr * lim) * inv
    cp_b(1).wait()
    mm1_cols(0, b_off[1], b_off[2], 2)
    cp_b(2).wait()
    mm1_cols(0, b_off[2], b_off[3], 2)
    cp_b(3).wait()
    cp_x(2).wait()
    ln(2, True)
    mm1_cols(0, b_off[3], b_off[4], 2)
    hr = jnp.zeros((8, 128), f32)
    hi = jnp.zeros((8, 128), f32)
    mm1_cols(2, 0, 2 * P)
    hr, hi = scan(0, hr, hi)
    cp_c[0].wait()
    cp_c[1].wait()
    for jj in range(3, N):
        cp_x(jj).wait()
    ln(3, True)
    ln(4, True)
    mm2(0)
    hr, hi = scan(1, hr, hi)
    cp_o(0).start()
    ln(5, True)
    ln(6, True)
    mm1_cols(3, 0, 2 * P)
    hr, hi = scan(2, hr, hi)
    ln(7, True)
    mm2(1)
    cp_o(1).start()
    mm1_cols(4, 0, 2 * P)
    hr, hi = scan(3, hr, hi)
    top2()
    mm2(2)
    cp_o(2).start()
    cp_w[0].wait()
    cp_w[1].wait()
    gu = gu_units()
    dn = down_units()
    _interleave(mm1_units(5), gu[0:32])
    hr, hi = scan(4, hr, hi)
    _interleave(mm2_units(3), gu[32:64])
    cp_o(3).start()
    _interleave(mm1_units(6), gu[64:96])
    hr, hi = scan(5, hr, hi)
    _interleave(mm2_units(4), gu[96:112])
    cp_o(4).start()
    cp_w[2].wait()
    _interleave(mm1_units(7), dn[0:32])
    hr, hi = scan(6, hr, hi)
    _interleave(mm2_units(5), dn[32:56])
    for jj in range(5):
        cp_o(jj).wait()
    finish = patch(5)
    cp_o(5).start()
    mm2(6)
    hr, hi = scan(7, hr, hi)
    cp_o(6).start()
    last = mm2_units(7)
    cp_l = [pltpu.make_async_copy(out_v.at[7 * T:8 * T, q * 128:(q + 1) * 128],
                                  out_hbm.at[7 * T:8 * T, q * 128:(q + 1) * 128], sem_l.at[q]) for q in range(8)]
    for q in range(8):
        for u in last[4 * q:4 * q + 4]:
            u()
        cp_l[q].start()
    finish()
    for jj in range(5, N - 1):
        cp_o(jj).wait()
    for c in cp_l:
        c.wait()


@jax.jit
def pallas_parallel_sum__ssm_conv_s5__moe_arch_mod__prompt_kernel(A_x, A_Lambda_re, A_Lambda_im, A_B_re, A_B_im, A_C_re, A_C_im, A_log_dt, A_Dskip,
              B_x, B_w_r, B_w_gate, B_w_up, B_w_down):
    x = A_x.reshape(L, D)
    s8 = lambda v: v.reshape(8, 128)
    any_spec = pl.BlockSpec(memory_space=pl.ANY)
    out = pl.pallas_call(
        _kernel,
        out_shape=jax.ShapeDtypeStruct((L, D), f32),
        in_specs=[any_spec] * 13,
        out_specs=any_spec,
        scratch_shapes=[
            pltpu.VMEM((L, D), bf16),
            pltpu.VMEM((L // 2, D), jnp.uint32),
            pltpu.VMEM((2 * P, D), bf16),
            pltpu.VMEM((D, P), bf16),
            pltpu.VMEM((D, P), bf16),
            pltpu.VMEM((D, F), bf16),
            pltpu.VMEM((D, F), bf16),
            pltpu.VMEM((F, D), bf16),
            pltpu.VMEM((L, D), f32),
            pltpu.VMEM((5, 8, 128), bf16),
            pltpu.VMEM((16, F), bf16),
            pltpu.VMEM((8 * TS, 128), f32),
            pltpu.VMEM((8 * TS, 128), f32),
            pltpu.VMEM((8 * TS, 128), f32),
            pltpu.VMEM((8 * TH, 128), jnp.uint32),
            pltpu.VMEM((8 * TH, 128), jnp.uint32),
            pltpu.SemaphoreType.DMA((N,)),
            pltpu.SemaphoreType.DMA((len(B_PIECES),)),
            pltpu.SemaphoreType.DMA((2,)),
            pltpu.SemaphoreType.DMA((3,)),
            pltpu.SemaphoreType.DMA((N,)),
            pltpu.SemaphoreType.DMA((5,)),
            pltpu.SemaphoreType.DMA((2,)),
            pltpu.SemaphoreType.REGULAR,
            pltpu.SemaphoreType.DMA((8,)),
        ],
        compiler_params=pltpu.CompilerParams(vmem_limit_bytes=110 * 1024 * 1024),
    )(x, s8(A_Lambda_re), s8(A_Lambda_im), s8(A_log_dt), s8(A_Dskip), s8(B_w_r),
      A_B_re, A_B_im, A_C_re, A_C_im, B_w_gate, B_w_up, B_w_down)
    return out.reshape(1, L, D)
```

```python
import jax
import jax.numpy as jnp
from jax import lax
import jax.experimental.pallas as pl
import jax.experimental.pallas.tpu as pltpu

L = 2048
D = 1024
P = 1024
F = 3584
T = 256
N = L // T
TS = 2 * T + 4
TH = T + 4
NT = (((1,), (1,)), ((), ()))
NN = (((1,), (0,)), ((), ()))
f32 = jnp.float32
bf16 = jnp.bfloat16
u32 = jnp.uint32
EPS_BF16 = 1.0013580322265625e-05
B_PIECES = ((0, 1), (1, 2), (2, 4), (4, 6), (6, 8))
LNG = 16
KU = 512
SCAN_SEGS = 16
NPATCH = 5


def _rb(v):
    return v.astype(bf16).astype(f32)


def _row(v8):
    return jnp.concatenate([v8[j:j + 1, :] for j in range(8)], axis=1)


def _dot(a, b, dims):
    return lax.dot_general(a, b, dims, preferred_element_type=f32)


def _zero_f(v):
    return jnp.where(v > jnp.inf, 1.0, 0.0)


def _gate(lhs_u32, deps):
    if not deps:
        return lhs_u32
    z = None
    for d in deps:
        zi = jnp.where(d > jnp.inf, jnp.uint32(1), jnp.uint32(0))
        z = zi if z is None else z | zi
    z = jnp.concatenate([z] * (lhs_u32.shape[1] // 128), axis=1)
    if lhs_u32.shape[0] == 8:
        return lhs_u32 | z
    return jnp.concatenate([lhs_u32[0:8, :] | z, lhs_u32[8:, :]], axis=0)


def _run(main, streams=(), hooks=None):
    hooks = hooks or {}
    at = {}
    for tasks, first, last, lag in streams:
        n = len(tasks)
        for t, task in enumerate(tasks):
            at.setdefault(first + t * (last - first) // n, []).append((task, lag))
    pending = {}
    for i, m in enumerate(main):
        tok = m(pending.pop(i, []))
        for task, lag in at.get(i, []):
            o = task(tok)
            if o is not None:
                pending.setdefault(i + lag, []).append(o)
        for h in hooks.get(i, []):
            h()


def _kernel(x_hbm, lre_hbm, lim_hbm, ldt_hbm, dsk_hbm, wr_hbm, bre_hbm, bim_hbm, cre_hbm, cim_hbm,
            wg_hbm, wu_hbm, wd_hbm, out_hbm,
            x_v, xn_v, b_v, cre_v, cim_v, wg_v, wu_v, wd_v, out_v, sm_v, act_v, *rest):
    S = rest[0:N]
    H = rest[N:2 * N]
    sem_x, sem_b, sem_c, sem_w, sem_o, sem_s, sem_f, sem_l = rest[2 * N:]

    def cp_x(j):
        return pltpu.make_async_copy(x_hbm.at[j * T:(j + 1) * T, :], x_v.at[j * T:(j + 1) * T, :], sem_x.at[j])

    def cp_b(p):
        k0, k1 = B_PIECES[p]
        return [pltpu.make_async_copy(src.at[k0:k1], b_v.at[k0:k1, c], sem_b.at[2 * p + c])
                for c, src in enumerate((bre_hbm, bim_hbm))]

    cp_c = [pltpu.make_async_copy(cre_hbm, cre_v, sem_c.at[0]), pltpu.make_async_copy(cim_hbm, cim_v, sem_c.at[1])]
    cp_w = [pltpu.make_async_copy(wg_hbm, wg_v, sem_w.at[0]), pltpu.make_async_copy(wu_hbm, wu_v, sem_w.at[1]),
            pltpu.make_async_copy(wd_hbm, wd_v, sem_w.at[2])]
    cp_s = [pltpu.make_async_copy(h, sm_v.at[i], sem_s.at[i])
            for i, h in enumerate((lre_hbm, lim_hbm, ldt_hbm, dsk_hbm, wr_hbm))]

    def cp_o(j):
        return pltpu.make_async_copy(out_v.at[j * T:(j + 1) * T, :], out_hbm.at[j * T:(j + 1) * T, :], sem_o.at[j])

    order = (cp_s + [cp_x(0)] + cp_b(0) + [cp_x(1)] + cp_b(1) + cp_b(2) + cp_b(3) + [cp_x(2)] + cp_b(4) + cp_c
             + [cp_x(jj) for jj in range(3, N)] + cp_w)
    for c in order:
        c.start()
        pl.semaphore_signal(sem_f, 1)
        pl.semaphore_wait(sem_f, 1)

    for c in cp_s:
        c.wait()
    lre = sm_v[0].astype(f32)
    lim = sm_v[1].astype(f32)
    dt = _rb(jnp.exp(sm_v[2].astype(f32)))
    mag = jnp.exp(dt * lre)
    ang = dt * lim
    ar = mag * jnp.cos(ang)
    ai = mag * jnp.sin(ang)
    nr = ar - 1.0
    inv = 2.0 / (lre * lre + lim * lim)
    fr = (nr * lre + ai * lim) * inv
    fi = (ai * lre - nr * lim) * inv
    dsk1 = _row(sm_v[3].astype(f32)) + 1.0
    wr = _row(sm_v[4].astype(f32))

    def x_f32(r0, tok):
        xa = x_v[r0:r0 + 8, :].astype(f32)
        if tok is not None:
            xa = jnp.concatenate([xa[:, 0:128] + _zero_f(tok), xa[:, 128:]], axis=1)
        return jnp.concatenate([xa, x_v[r0 + 8:r0 + 16, :].astype(f32)], axis=0)

    def ln_group(r0, fast, tok):
        x = x_f32(r0, tok)
        mu = jnp.sum(x, axis=-1, keepdims=True) * (1.0 / D)
        mb = _rb(mu)
        xc = x - mb
        ex2 = jnp.sum(xc * xc, axis=-1, keepdims=True) * (1.0 / D)
        dm = mu - mb
        var = jnp.maximum(ex2 - dm * dm, 0.0)
        den = _rb(jnp.sqrt(_rb(_rb(var) + EPS_BF16)))
        xn = xc * (1.0 / den)
        xn_v[r0 // 2:(r0 + LNG) // 2, :] = pltpu.bitcast(xn.astype(bf16), u32)
        if fast:
            return None
        return r_part(r0, xn)

    racc = {"v": jnp.zeros((LNG, 128), f32)}
    lane_iota = lax.broadcasted_iota(jnp.int32, (LNG, 128), 1)

    def r_part(r0, xn):
        xw = xn * wr
        ps = xw[:, 0:128]
        for c in range(1, 8):
            ps = ps + xw[:, c * 128:(c + 1) * 128]
        r = _rb(jnp.sum(ps, axis=-1, keepdims=True))
        racc["v"] = jnp.where(lane_iota == r0 // LNG, r, racc["v"])
        return ps[0:8, :] + ps[8:16, :]

    def ln_fast(j):
        for g in range(T // LNG):
            ln_group(j * T + g * LNG, True, None)

    def ln_tasks(j):
        return [(lambda tok, r0=j * T + g * LNG: ln_group(r0, False, tok)) for g in range(T // LNG)]

    def rest_group(r0, tok):
        xu = xn_v[r0 // 2:(r0 + LNG) // 2, :]
        xn = pltpu.bitcast(_gate(xu, [tok]), bf16).astype(f32)
        return r_part(r0, xn)

    def rest_tasks(j):
        return [(lambda tok, r0=j * T + g * LNG: rest_group(r0, tok)) for g in range(T // LNG)]

    def xn_u32(r0, r1, c0, c1):
        return xn_v[r0 // 2:r1 // 2, c0:c1]

    def s_store(j, k, re, im):
        frk = fr[k:k + 1, :]
        fik = fi[k:k + 1, :]
        S[j][pl.ds(k * TS, T, stride=2), :] = frk * re - fik * im
        S[j][pl.ds(k * TS + 1, T, stride=2), :] = frk * im + fik * re

    def mm1_units(j, nchunk=1, k0=0, k1=8):
        acc = {}

        def unit(k, c, h):
            def run(deps):
                lhs = _gate(xn_u32(j * T, (j + nchunk) * T, h * KU, (h + 1) * KU), deps)
                part = _dot(pltpu.bitcast(lhs, bf16), b_v[k, c, :, h * KU:(h + 1) * KU], NT)
                acc[(k, c)] = part if h == 0 else acc[(k, c)] + part
                if c == 1 and h == 1:
                    re = acc.pop((k, 0))
                    im = acc.pop((k, 1))
                    for cc in range(nchunk):
                        s_store(j + cc, k, re[cc * T:(cc + 1) * T], im[cc * T:(cc + 1) * T])
                return part[0:8, :]
            return run
        return [unit(k, c, h) for k in range(k0, k1) for c in range(2) for h in range(D // KU)]

    hst = {"r": jnp.zeros((8, 128), f32), "i": jnp.zeros((8, 128), f32)}

    def scan_seg(j, t0, t1, tok):
        s = S[j]
        h = H[j]
        hr, hi = hst["r"], hst["i"]
        if tok is not None:
            hr = hr + _zero_f(tok)
        for t2 in range(t0 // 2, t1 // 2):
            outs = []
            for t in (2 * t2, 2 * t2 + 1):
                ur = s[pl.ds(2 * t, 8, stride=TS), :]
                ui = s[pl.ds(2 * t + 1, 8, stride=TS), :]
                nr_ = ar * hr - ai * hi + ur
                ni_ = ar * hi + ai * hr + ui
                hr, hi = nr_, ni_
                outs.append((hr, hi))
            h[pl.ds(2 * t2, 8, stride=TH), :] = pltpu.pack_elementwise(
                [outs[0][0], outs[1][0]], packed_dtype=bf16)
            h[pl.ds(2 * t2 + 1, 8, stride=TH), :] = pltpu.pack_elementwise(
                [outs[0][1], outs[1][1]], packed_dtype=bf16)
        hst["r"], hst["i"] = hr, hi
        return hr

    def scan_tasks(j, nseg=SCAN_SEGS):
        w = T // nseg
        return [(lambda tok, a=a: scan_seg(j, a, a + w, tok)) for a in range(0, T, w)]

    def h_u32(j, k):
        return H[j][pl.ds((k % 8) * TH + k // 8, T // 2, stride=2), :]

    def mm2_units(j):
        rows = slice(j * T, (j + 1) * T)
        acc = {}

        def unit(q, u):
            def run(deps):
                cols = slice(q * 128, (q + 1) * 128)
                ks = slice((u % 2) * KU, (u % 2 + 1) * KU)
                lhs = jnp.concatenate([h_u32(j, 4 * u + a) for a in range(4)], axis=1)
                lhs = pltpu.bitcast(_gate(lhs, deps), bf16)
                cw = cre_v if u < 2 else cim_v
                part = _dot(lhs, cw[cols, ks], NT)
                if u == 0:
                    acc[q] = part
                elif u == 1:
                    acc[q] = acc[q] + part
                elif u == 2:
                    acc[q] = acc[q] - part
                else:
                    xq = x_v[rows, cols].astype(f32)
                    xnq = pltpu.bitcast(xn_v[j * T // 2:(j + 1) * T // 2, cols], bf16).astype(f32)
                    o = (acc.pop(q) - part) + (xq + xnq * dsk1[:, cols])
                    if j >= NPATCH:
                        rid = lax.broadcasted_iota(jnp.int32, (T, 128), 0) + j * T
                        for k, i in enumerate(st["i"]):
                            o = o + jnp.where(rid == i, st["upd"][k:k + 1, cols], 0.0)
                    out_v[rows, cols] = o
                return part[0:8, :]
            return run
        return [unit(q, u) for q in range(8) for u in range(4)]

    st = {}

    def top2():
        vals = racc["v"]
        idxs = (lane_iota * LNG + lax.broadcasted_iota(jnp.int32, (LNG, 128), 0)).astype(f32)

        def amax(v):
            return jnp.max(jnp.max(v, axis=1, keepdims=True), axis=0, keepdims=True)

        def amin(v):
            return jnp.min(jnp.min(v, axis=1, keepdims=True), axis=0, keepdims=True)

        m1 = amax(vals)
        i1f = amin(jnp.where(vals == m1, idxs, float(L)))
        vals2 = jnp.where(idxs == i1f, -jnp.inf, vals)
        m2 = amax(vals2)
        i2f = amin(jnp.where(vals2 == m2, idxs, float(L)))
        i1 = jnp.clip(jnp.min(i1f).astype(jnp.int32), 0, L - 1)
        i2 = jnp.clip(jnp.min(i2f).astype(jnp.int32), 0, L - 1)

        def gather(i):
            base = pl.multiple_of((i // 16) * 8, 8)
            tile = pltpu.bitcast(xn_v[pl.ds(base, 8), :], bf16).astype(f32)
            sel = lax.broadcasted_iota(jnp.int32, (16, D), 0) == (i % 16)
            return jnp.sum(jnp.where(sel, tile, 0.0), axis=0, keepdims=True)

        rid = lax.broadcasted_iota(jnp.int32, (16, D), 0)
        xs = jnp.where(rid == 0, gather(i1), jnp.where(rid == 1, gather(i2), 0.0)).astype(bf16)
        st["xs"] = pltpu.bitcast(xs, u32)
        st["i"] = (i1, i2)
        st["m"] = (m1, m2)

    def gu_units():
        def unit(k, w, h):
            def run(dep):
                cols = slice(k * 128, (k + 1) * 128)
                ks = slice(h * KU, (h + 1) * KU)
                lhs = pltpu.bitcast(_gate(st["xs"][:, ks], [dep]), bf16)
                part = _dot(lhs, (wg_v, wu_v)[w][ks, cols], NN)
                key = ("gu", k, w)
                st[key] = part if h == 0 else st[key] + part
                if w == 1 and h == 1:
                    g = st.pop(("gu", k, 0))
                    u = st.pop(("gu", k, 1))
                    act_v[:, cols] = pltpu.bitcast((g * jax.nn.sigmoid(g) * u).astype(bf16), u32)
                return part[0:8, :]
            return run
        return [unit(k, w, h) for k in range(F // 128) for w in range(2) for h in range(2)]

    def down_units():
        def unit(q, u):
            def run(dep):
                cols = slice(q * 128, (q + 1) * 128)
                ks = slice(u * KU, (u + 1) * KU)
                lhs = pltpu.bitcast(_gate(act_v[:, ks], [dep]), bf16)
                part = _dot(lhs, wd_v[ks, cols], NN)
                key = ("y", q)
                st[key] = part if u == 0 else st[key] + part
                return part[0:8, :]
            return run
        return [unit(q, u) for q in range(8) for u in range(F // KU)]

    def patch():
        m1, m2 = st["m"]
        y = jnp.concatenate([st[("y", q)] for q in range(8)], axis=1)
        rid = lax.broadcasted_iota(jnp.int32, (16, D), 0)
        rs = jnp.where(rid == 0, m1, m2)
        st["upd"] = y * jax.nn.sigmoid(rs)
        for k, i in enumerate(st["i"]):
            g0 = pl.multiple_of(jnp.minimum(i // 8, NPATCH * T // 8 - 1) * 8, 8)
            sel = lax.broadcasted_iota(jnp.int32, (8, D), 0) == (i - g0)
            blk = out_v[pl.ds(g0, 8), :]
            out_v[pl.ds(g0, 8), :] = blk + jnp.where(sel, st["upd"][k:k + 1, :], 0.0)

    def wait_all(cs):
        for c in cs:
            c.wait()

    cp_x(0).wait()
    ln_fast(0)
    wait_all(cp_b(0))
    _run(mm1_units(0, 1, *B_PIECES[0]))
    cp_x(1).wait()
    ln_fast(1)
    wait_all(cp_b(1))
    _run(mm1_units(1, 1, *B_PIECES[0]) + mm1_units(0, 2, *B_PIECES[1]))
    wait_all(cp_b(2))
    _run(mm1_units(0, 2, *B_PIECES[2]))
    wait_all(cp_b(3))
    _run(mm1_units(0, 2, *B_PIECES[3]))
    wait_all(cp_b(4) + [cp_x(2)])
    _run(mm1_units(0, 2, *B_PIECES[4]) + mm1_units(2),
         [(ln_tasks(2), 0, 6, 2), (rest_tasks(0) + rest_tasks(1), 8, 24, 2), (scan_tasks(0), 10, 38, 2)])
    wait_all(cp_c + [cp_x(jj) for jj in range(3, N)])
    _run(mm2_units(0) + mm1_units(3) + mm2_units(1) + mm1_units(4),
         [(ln_tasks(3), 0, 20, 3), (scan_tasks(1), 0, 30, 2),
          (ln_tasks(4), 20, 40, 3), (scan_tasks(2), 32, 62, 2),
          (ln_tasks(5), 40, 60, 3),
          (ln_tasks(6), 60, 80, 3), (scan_tasks(3), 66, 94, 2),
          (ln_tasks(7), 80, 100, 3)],
         {106: [top2]})
    wait_all(cp_w[0:2])
    gu = gu_units()
    dn = down_units()
    _run(mm2_units(2) + mm1_units(5) + mm2_units(3),
         [(gu[0:96], 0, 96, 2), (scan_tasks(4), 0, 30, 2), (scan_tasks(5), 66, 94, 2)])
    cp_w[2].wait()
    cp_l = [pltpu.make_async_copy(out_v.at[7 * T:8 * T, q * 128:(q + 1) * 128],
                                  out_hbm.at[7 * T:8 * T, q * 128:(q + 1) * 128], sem_l.at[q]) for q in range(8)]
    hooks = {78: [patch] + [cp_o(jj).start for jj in range(5)], 127: [cp_o(5).start], 159: [cp_o(6).start]}
    for q in range(8):
        hooks[160 + 4 * q + 3] = [cp_l[q].start]
    _run(mm1_units(6) + mm2_units(4) + mm1_units(7) + mm2_units(5) + mm2_units(6) + mm2_units(7),
         [(gu[96:112], 0, 16, 2), (dn, 18, 74, 2), (scan_tasks(6), 34, 62, 2), (scan_tasks(7), 98, 126, 2)], hooks)
    for jj in range(N - 1):
        cp_o(jj).wait()
    for c in cp_l:
        c.wait()


@jax.jit
def pallas_parallel_sum__ssm_conv_s5__moe_arch_mod__prompt_kernel(A_x, A_Lambda_re, A_Lambda_im, A_B_re, A_B_im, A_C_re, A_C_im, A_log_dt, A_Dskip,
              B_x, B_w_r, B_w_gate, B_w_up, B_w_down):
    x = A_x.reshape(L, D)
    s8 = lambda v: v.reshape(8, 128)
    any_spec = pl.BlockSpec(memory_space=pl.ANY)
    out = pl.pallas_call(
        _kernel,
        out_shape=jax.ShapeDtypeStruct((L, D), f32),
        in_specs=[any_spec] * 13,
        out_specs=any_spec,
        scratch_shapes=[
            pltpu.VMEM((L, D), bf16),
            pltpu.VMEM((L // 2, D), u32),
            pltpu.VMEM((8, 2, 128, D), bf16),
            pltpu.VMEM((D, P), bf16),
            pltpu.VMEM((D, P), bf16),
            pltpu.VMEM((D, F), bf16),
            pltpu.VMEM((D, F), bf16),
            pltpu.VMEM((F, D), bf16),
            pltpu.VMEM((L, D), f32),
            pltpu.VMEM((5, 8, 128), bf16),
            pltpu.VMEM((8, F), u32),
        ] + [pltpu.VMEM((8 * TS, 128), f32) for _ in range(N)]
          + [pltpu.VMEM((8 * TH, 128), u32) for _ in range(N)] + [
            pltpu.SemaphoreType.DMA((N,)),
            pltpu.SemaphoreType.DMA((2 * len(B_PIECES),)),
            pltpu.SemaphoreType.DMA((2,)),
            pltpu.SemaphoreType.DMA((3,)),
            pltpu.SemaphoreType.DMA((N,)),
            pltpu.SemaphoreType.DMA((5,)),
            pltpu.SemaphoreType.REGULAR,
            pltpu.SemaphoreType.DMA((8,)),
        ],
        compiler_params=pltpu.CompilerParams(vmem_limit_bytes=110 * 1024 * 1024),
    )(x, s8(A_Lambda_re), s8(A_Lambda_im), s8(A_log_dt), s8(A_Dskip), s8(B_w_r),
      A_B_re.reshape(8, 128, D), A_B_im.reshape(8, 128, D), A_C_re, A_C_im, B_w_gate, B_w_up, B_w_down)
    return out.reshape(1, L, D)
```

```python
import jax
import jax.numpy as jnp
from jax import lax
import jax.experimental.pallas as pl
import jax.experimental.pallas.tpu as pltpu

L = 2048
D = 1024
P = 1024
F = 3584
T = 256
N = L // T
TS = 2 * T + 4
TH = T + 4
NT = (((1,), (1,)), ((), ()))
NN = (((1,), (0,)), ((), ()))
f32 = jnp.float32
bf16 = jnp.bfloat16
u32 = jnp.uint32
EPS_BF16 = 1.0013580322265625e-05
B_PIECES = ((0, 1), (1, 2), (2, 4), (4, 6), (6, 8))
LNG = 16
KU = 512
SCAN_SEGS = 16
NPATCH = 5


def _rb(v):
    return v.astype(bf16).astype(f32)


def _row(v8):
    return jnp.concatenate([v8[j:j + 1, :] for j in range(8)], axis=1)


def _dot(a, b, dims):
    return lax.dot_general(a, b, dims, preferred_element_type=f32)


def _zero_f(v):
    return jnp.where(v > jnp.inf, 1.0, 0.0)


def _pack2(a, b):
    ua = lax.bitcast_convert_type(a, u32) + jnp.uint32(0x8000)
    ub = lax.bitcast_convert_type(b, u32) + jnp.uint32(0x8000)
    return (ua >> 16) | (ub & jnp.uint32(0xFFFF0000))


def _gate(lhs_u32, deps):
    if not deps:
        return lhs_u32
    z = None
    for d in deps:
        zi = jnp.where(d > jnp.inf, jnp.uint32(1), jnp.uint32(0))
        z = zi if z is None else z | zi
    z = jnp.concatenate([z] * (lhs_u32.shape[1] // 128), axis=1)
    if lhs_u32.shape[0] == 8:
        return lhs_u32 | z
    return jnp.concatenate([lhs_u32[0:8, :] | z, lhs_u32[8:, :]], axis=0)


def _gate_f(lhs, dep):
    z = _zero_f(dep)
    return lhs + jnp.concatenate([z] * (lhs.shape[1] // 128), axis=1)


def _run(main, streams=(), hooks=None):
    hooks = hooks or {}
    at = {}
    for tasks, first, last, lag in streams:
        n = len(tasks)
        for t, task in enumerate(tasks):
            at.setdefault(first + t * (last - first) // n, []).append((task, lag))
    pending = {}
    for i, m in enumerate(main):
        tok = m(pending.pop(i, []))
        for task, lag in at.get(i, []):
            o = task(tok)
            if o is not None:
                pending.setdefault(i + lag, []).append(o)
        for h in hooks.get(i, []):
            h()


def _kernel(x_hbm, lre_hbm, lim_hbm, ldt_hbm, dsk_hbm, wr_hbm, bre_hbm, bim_hbm, cre_hbm, cim_hbm,
            wg_hbm, wu_hbm, wd_hbm, out_hbm,
            x_v, xn_v, b_v, cre_v, cim_v, wg_v, wu_v, wd_v, out_v, sm_v, act_v, *rest):
    S = rest[0:N]
    H = rest[N:2 * N]
    sem, sem_f = rest[2 * N:]
    SEM_S, SEM_X0, SEM_X1, SEM_B0, SEM_C, SEM_W, SEM_D, SEM_O = 0, 1, 2, 3, 8, 9, 10, 11

    def cp_x(j):
        return pltpu.make_async_copy(x_hbm.at[j * T:(j + 1) * T, :], x_v.at[j * T:(j + 1) * T, :],
                                     sem.at[(SEM_X0, SEM_X1, SEM_B0 + 4)[j] if j < 3 else SEM_C])

    def cp_b(p):
        k0, k1 = B_PIECES[p]
        return [pltpu.make_async_copy(src.at[k0:k1], b_v.at[k0:k1, c], sem.at[SEM_B0 + p])
                for c, src in enumerate((bre_hbm, bim_hbm))]

    cp_c = [pltpu.make_async_copy(cre_hbm, cre_v, sem.at[SEM_C]), pltpu.make_async_copy(cim_hbm, cim_v, sem.at[SEM_C])]
    cp_w = [pltpu.make_async_copy(wg_hbm, wg_v, sem.at[SEM_W]), pltpu.make_async_copy(wu_hbm, wu_v, sem.at[SEM_W]),
            pltpu.make_async_copy(wd_hbm, wd_v, sem.at[SEM_D])]
    cp_s = [pltpu.make_async_copy(h, sm_v.at[i], sem.at[SEM_S])
            for i, h in enumerate((lre_hbm, lim_hbm, ldt_hbm, dsk_hbm, wr_hbm))]

    def cp_o(j):
        return pltpu.make_async_copy(out_v.at[j * T:(j + 1) * T, :], out_hbm.at[j * T:(j + 1) * T, :], sem.at[SEM_O])

    order = ([cp_x(0)] + cp_s + cp_b(0) + [cp_x(1)] + cp_b(1) + cp_b(2) + cp_b(3) + [cp_x(2)] + cp_b(4) + cp_c
             + [cp_x(jj) for jj in range(3, N)] + cp_w)
    for c in order:
        c.start()
        pl.semaphore_signal(sem_f, 1)
        pl.semaphore_wait(sem_f, 1)

    cp_x(0).wait()
    for c in cp_s:
        c.wait()
    lre = sm_v[0].astype(f32)
    lim = sm_v[1].astype(f32)
    dt = _rb(jnp.exp(sm_v[2].astype(f32)))
    mag = jnp.exp(dt * lre)
    ang = dt * lim
    ar = mag * jnp.cos(ang)
    ai = mag * jnp.sin(ang)
    nr = ar - 1.0
    inv = 2.0 / (lre * lre + lim * lim)
    fr = (nr * lre + ai * lim) * inv
    fi = (ai * lre - nr * lim) * inv
    dsk1 = _row(sm_v[3].astype(f32)) + 1.0
    wr = _row(sm_v[4].astype(f32))

    def x_f32(r0, tok):
        xa = x_v[r0:r0 + 8, :].astype(f32)
        if tok is not None:
            xa = jnp.concatenate([xa[:, 0:128] + _zero_f(tok), xa[:, 128:]], axis=1)
        return jnp.concatenate([xa, x_v[r0 + 8:r0 + 16, :].astype(f32)], axis=0)

    def ln_group(r0, fast, tok):
        x = x_f32(r0, tok)
        mu = jnp.sum(x, axis=-1, keepdims=True) * (1.0 / D)
        mb = _rb(mu)
        xc = x - mb
        ex2 = jnp.sum(xc * xc, axis=-1, keepdims=True) * (1.0 / D)
        dm = mu - mb
        var = jnp.maximum(ex2 - dm * dm, 0.0)
        den = _rb(jnp.sqrt(_rb(_rb(var) + EPS_BF16)))
        xn = xc * (1.0 / den)
        xn_v[r0 // 2:(r0 + LNG) // 2, :] = pltpu.bitcast(xn.astype(bf16), u32)
        if fast:
            return None
        return r_part(r0, xn)

    racc = {"v": jnp.zeros((LNG, 128), f32)}
    lane_iota = lax.broadcasted_iota(jnp.int32, (LNG, 128), 1)

    def r_part(r0, xn):
        xw = xn * wr
        ps = xw[:, 0:128]
        for c in range(1, 8):
            ps = ps + xw[:, c * 128:(c + 1) * 128]
        r = _rb(jnp.sum(ps, axis=-1, keepdims=True))
        racc["v"] = jnp.where(lane_iota == r0 // LNG, r, racc["v"])
        return ps[0:8, :] + ps[8:16, :]

    def ln_fast(j):
        for g in range(T // LNG):
            ln_group(j * T + g * LNG, True, None)

    def ln_tasks(j):
        return [(lambda tok, r0=j * T + g * LNG: ln_group(r0, False, tok)) for g in range(T // LNG)]

    def rest_group(r0, tok):
        xu = xn_v[r0 // 2:(r0 + LNG) // 2, :]
        xn = pltpu.bitcast(_gate(xu, [tok]), bf16).astype(f32)
        return r_part(r0, xn)

    def rest_tasks(j):
        return [(lambda tok, r0=j * T + g * LNG: rest_group(r0, tok)) for g in range(T // LNG)]

    def xn_u32(r0, r1, c0, c1):
        return xn_v[r0 // 2:r1 // 2, c0:c1]

    def s_store(j, k, re, im):
        frk = fr[k:k + 1, :]
        fik = fi[k:k + 1, :]
        S[j][pl.ds(k * TS, T, stride=2), :] = frk * re - fik * im
        S[j][pl.ds(k * TS + 1, T, stride=2), :] = frk * im + fik * re

    def mm1_units(j, nchunk=1, k0=0, k1=8):
        acc = {}

        def unit(k, c, h):
            def run(deps):
                lhs = _gate(xn_u32(j * T, (j + nchunk) * T, h * KU, (h + 1) * KU), deps)
                part = _dot(pltpu.bitcast(lhs, bf16), b_v[k, c, :, h * KU:(h + 1) * KU], NT)
                acc[(k, c)] = part if h == 0 else acc[(k, c)] + part
                if c == 1 and h == 1:
                    re = acc.pop((k, 0))
                    im = acc.pop((k, 1))
                    for cc in range(nchunk):
                        s_store(j + cc, k, re[cc * T:(cc + 1) * T], im[cc * T:(cc + 1) * T])
                return part[0:8, :]
            return run
        return [unit(k, c, h) for k in range(k0, k1) for c in range(2) for h in range(D // KU)]

    hst = {"r": jnp.zeros((8, 128), f32), "i": jnp.zeros((8, 128), f32)}

    def scan_seg(j, t0, t1, tok):
        s = S[j]
        h = H[j]
        hr, hi = hst["r"], hst["i"]
        if tok is not None:
            hr = hr + _zero_f(tok)
        for t2 in range(t0 // 2, t1 // 2):
            outs = []
            for t in (2 * t2, 2 * t2 + 1):
                ur = s[pl.ds(2 * t, 8, stride=TS), :]
                ui = s[pl.ds(2 * t + 1, 8, stride=TS), :]
                nr_ = ar * hr - ai * hi + ur
                ni_ = ar * hi + ai * hr + ui
                hr, hi = nr_, ni_
                outs.append((hr, hi))
            h[pl.ds(2 * t2, 8, stride=TH), :] = _pack2(outs[0][0], outs[1][0])
            h[pl.ds(2 * t2 + 1, 8, stride=TH), :] = _pack2(outs[0][1], outs[1][1])
        hst["r"], hst["i"] = hr, hi
        return hr

    def scan_tasks(j, nseg=SCAN_SEGS):
        w = T // nseg
        return [(lambda tok, a=a: scan_seg(j, a, a + w, tok)) for a in range(0, T, w)]

    def h_u32(j, k):
        return H[j][pl.ds((k % 8) * TH + k // 8, T // 2, stride=2), :]

    def mm2_units(j):
        rows = slice(j * T, (j + 1) * T)
        acc = {}

        def unit(q, u):
            def run(deps):
                cols = slice(q * 128, (q + 1) * 128)
                ks = slice((u % 2) * KU, (u % 2 + 1) * KU)
                lhs = jnp.concatenate([h_u32(j, 4 * u + a) for a in range(4)], axis=1)
                lhs = pltpu.bitcast(_gate(lhs, deps), bf16)
                cw = cre_v if u < 2 else cim_v
                part = _dot(lhs, cw[cols, ks], NT)
                if u == 0:
                    acc[q] = part
                elif u == 1:
                    acc[q] = acc[q] + part
                elif u == 2:
                    acc[q] = acc[q] - part
                else:
                    xq = x_v[rows, cols].astype(f32)
                    xnq = pltpu.bitcast(xn_v[j * T // 2:(j + 1) * T // 2, cols], bf16).astype(f32)
                    o = (acc.pop(q) - part) + (xq + xnq * dsk1[:, cols])
                    if j >= NPATCH:
                        rid = lax.broadcasted_iota(jnp.int32, (T, 128), 0) + j * T
                        for k, i in enumerate(st["i"]):
                            o = o + jnp.where(rid == i, st["upd"][k:k + 1, cols], 0.0)
                    out_v[rows, cols] = o
                return part[0:8, :]
            return run
        return [unit(q, u) for q in range(8) for u in range(4)]

    st = {}

    def top2():
        vals = racc["v"]
        idxs = (lane_iota * LNG + lax.broadcasted_iota(jnp.int32, (LNG, 128), 0)).astype(f32)

        def amax(v):
            return jnp.max(jnp.max(v, axis=1, keepdims=True), axis=0, keepdims=True)

        def amin(v):
            return jnp.min(jnp.min(v, axis=1, keepdims=True), axis=0, keepdims=True)

        m1 = amax(vals)
        i1f = amin(jnp.where(vals == m1, idxs, float(L)))
        vals2 = jnp.where(idxs == i1f, -jnp.inf, vals)
        m2 = amax(vals2)
        i2f = amin(jnp.where(vals2 == m2, idxs, float(L)))
        i1 = jnp.clip(jnp.min(i1f).astype(jnp.int32), 0, L - 1)
        i2 = jnp.clip(jnp.min(i2f).astype(jnp.int32), 0, L - 1)

        def gather(i):
            base = pl.multiple_of((i // 16) * 8, 8)
            tile = pltpu.bitcast(xn_v[pl.ds(base, 8), :], bf16).astype(f32)
            sel = lax.broadcasted_iota(jnp.int32, (16, D), 0) == (i % 16)
            return jnp.sum(jnp.where(sel, tile, 0.0), axis=0, keepdims=True)

        rid = lax.broadcasted_iota(jnp.int32, (8, D), 0)
        st["xs"] = jnp.where(rid == 0, gather(i1), jnp.where(rid == 1, gather(i2), 0.0))
        st["i"] = (i1, i2)
        st["m"] = (m1, m2)

    def gu_units():
        def unit(k, w, h):
            def run(dep):
                cols = slice(k * 128, (k + 1) * 128)
                ks = slice(h * KU, (h + 1) * KU)
                lhs = _gate_f(st["xs"][:, ks], dep)
                part = _dot(lhs, (wg_v, wu_v)[w][ks, cols].astype(f32), NN)
                key = ("gu", k, w)
                st[key] = part if h == 0 else st[key] + part
                if w == 1 and h == 1:
                    g = st.pop(("gu", k, 0))
                    u = st.pop(("gu", k, 1))
                    act_v[:, cols] = _rb(g * jax.nn.sigmoid(g) * u)
                return part[0:8, :]
            return run
        return [unit(k, w, h) for k in range(F // 128) for w in range(2) for h in range(2)]

    def down_units():
        def unit(q, u):
            def run(dep):
                cols = slice(q * 128, (q + 1) * 128)
                ks = slice(u * KU, (u + 1) * KU)
                lhs = _gate_f(act_v[:, ks], dep)
                part = _dot(lhs, wd_v[ks, cols].astype(f32), NN)
                key = ("y", q)
                st[key] = part if u == 0 else st[key] + part
                return part[0:8, :]
            return run
        return [unit(q, u) for q in range(8) for u in range(F // KU)]

    def patch():
        m1, m2 = st["m"]
        y = jnp.concatenate([st[("y", q)] for q in range(8)], axis=1)
        rid = lax.broadcasted_iota(jnp.int32, (8, D), 0)
        rs = jnp.where(rid == 0, m1, m2)
        st["upd"] = y * jax.nn.sigmoid(rs)
        for k, i in enumerate(st["i"]):
            g0 = pl.multiple_of(jnp.minimum(i // 8, NPATCH * T // 8 - 1) * 8, 8)
            sel = lax.broadcasted_iota(jnp.int32, (8, D), 0) == (i - g0)
            blk = out_v[pl.ds(g0, 8), :]
            out_v[pl.ds(g0, 8), :] = blk + jnp.where(sel, st["upd"][k:k + 1, :], 0.0)

    def wait_all(cs):
        for c in cs:
            c.wait()

    ln_fast(0)
    wait_all(cp_b(0))
    _run(mm1_units(0, 1, *B_PIECES[0]))
    cp_x(1).wait()
    ln_fast(1)
    _run(mm1_units(1, 1, *B_PIECES[0]))
    wait_all(cp_b(1))
    _run(mm1_units(0, 2, *B_PIECES[1]))
    wait_all(cp_b(2))
    _run(mm1_units(0, 2, *B_PIECES[2]))
    wait_all(cp_b(3))
    _run(mm1_units(0, 2, *B_PIECES[3]))
    wait_all(cp_b(4) + [cp_x(2)])
    _run(mm1_units(0, 2, *B_PIECES[4]) + mm1_units(2),
         [(ln_tasks(2), 0, 6, 2), (rest_tasks(0) + rest_tasks(1), 8, 24, 2), (scan_tasks(0), 10, 38, 2)])
    wait_all(cp_c + [cp_x(jj) for jj in range(3, N)])
    _run(mm2_units(0) + mm1_units(3) + mm2_units(1) + mm1_units(4),
         [(ln_tasks(3), 0, 20, 3), (scan_tasks(1), 0, 30, 2),
          (ln_tasks(4), 20, 40, 3), (scan_tasks(2), 32, 62, 2),
          (ln_tasks(5), 40, 60, 3),
          (ln_tasks(6), 60, 80, 3), (scan_tasks(3), 66, 94, 2),
          (ln_tasks(7), 80, 100, 3)],
         {106: [top2]})
    wait_all(cp_w[0:2])
    gu = gu_units()
    dn = down_units()
    _run(mm2_units(2) + mm1_units(5) + mm2_units(3),
         [(gu[0:96], 0, 96, 2), (scan_tasks(4), 0, 30, 2), (scan_tasks(5), 66, 94, 2)])
    cp_w[2].wait()
    cp_l = [pltpu.make_async_copy(out_v.at[7 * T:8 * T, q * 128:(q + 1) * 128],
                                  out_hbm.at[7 * T:8 * T, q * 128:(q + 1) * 128], sem.at[SEM_O]) for q in range(8)]
    hooks = {78: [patch] + [cp_o(jj).start for jj in range(5)], 127: [cp_o(5).start], 159: [cp_o(6).start]}
    for q in range(8):
        hooks[160 + 4 * q + 3] = [cp_l[q].start]
    _run(mm1_units(6) + mm2_units(4) + mm1_units(7) + mm2_units(5) + mm2_units(6) + mm2_units(7),
         [(gu[96:112], 0, 16, 2), (dn, 18, 74, 2), (scan_tasks(6), 34, 62, 2), (scan_tasks(7), 98, 126, 2)], hooks)
    pltpu.make_async_copy(out_v, out_hbm, sem.at[SEM_O]).wait()


@jax.jit
def pallas_parallel_sum__ssm_conv_s5__moe_arch_mod__prompt_kernel(A_x, A_Lambda_re, A_Lambda_im, A_B_re, A_B_im, A_C_re, A_C_im, A_log_dt, A_Dskip,
              B_x, B_w_r, B_w_gate, B_w_up, B_w_down):
    x = A_x.reshape(L, D)
    s8 = lambda v: v.reshape(8, 128)
    any_spec = pl.BlockSpec(memory_space=pl.ANY)
    out = pl.pallas_call(
        _kernel,
        out_shape=jax.ShapeDtypeStruct((L, D), f32),
        in_specs=[any_spec] * 13,
        out_specs=any_spec,
        scratch_shapes=[
            pltpu.VMEM((L, D), bf16),
            pltpu.VMEM((L // 2, D), u32),
            pltpu.VMEM((8, 2, 128, D), bf16),
            pltpu.VMEM((D, P), bf16),
            pltpu.VMEM((D, P), bf16),
            pltpu.VMEM((D, F), bf16),
            pltpu.VMEM((D, F), bf16),
            pltpu.VMEM((F, D), bf16),
            pltpu.VMEM((L, D), f32),
            pltpu.VMEM((5, 8, 128), bf16),
            pltpu.VMEM((8, F), f32),
        ] + [pltpu.VMEM((9 * TS, 128), f32) for _ in range(N)]
          + [pltpu.VMEM((9 * TH, 128), u32) for _ in range(N)] + [
            pltpu.SemaphoreType.DMA((12,)),
            pltpu.SemaphoreType.REGULAR,
        ],
        compiler_params=pltpu.CompilerParams(vmem_limit_bytes=110 * 1024 * 1024),
    )(x, s8(A_Lambda_re), s8(A_Lambda_im), s8(A_log_dt), s8(A_Dskip), s8(B_w_r),
      A_B_re.reshape(8, 128, D), A_B_im.reshape(8, 128, D), A_C_re, A_C_im, B_w_gate, B_w_up, B_w_down)
    return out.reshape(1, L, D)
```

```python
import jax
import jax.numpy as jnp
from jax import lax
import jax.experimental.pallas as pl
import jax.experimental.pallas.tpu as pltpu

L = 2048
D = 1024
P = 1024
F = 3584
T = 256
N = L // T
TS = 2 * T + 4
TH = T + 4
NT = (((1,), (1,)), ((), ()))
NN = (((1,), (0,)), ((), ()))
f32 = jnp.float32
bf16 = jnp.bfloat16
u32 = jnp.uint32
EPS_BF16 = 1.0013580322265625e-05
B_PIECES = ((0, 1), (1, 2), (2, 4), (4, 6), (6, 8))
LNG = 16
KU = 512
SCAN_SEGS = 16
GU_LAG = 3
NPATCH = 5


def _rb(v):
    return v.astype(bf16).astype(f32)


def _row(v8):
    return jnp.concatenate([v8[j:j + 1, :] for j in range(8)], axis=1)


def _dot(a, b, dims):
    return lax.dot_general(a, b, dims, preferred_element_type=f32)


def _zero_f(v):
    return jnp.where(v > jnp.inf, 1.0, 0.0)


def _pack2(a, b):
    ua = lax.bitcast_convert_type(a, u32) + jnp.uint32(0x8000)
    ub = lax.bitcast_convert_type(b, u32) + jnp.uint32(0x8000)
    return (ua >> 16) | (ub & jnp.uint32(0xFFFF0000))


def _gate(lhs_u32, deps):
    if not deps:
        return lhs_u32
    z = None
    for d in deps:
        zi = jnp.where(d > jnp.inf, jnp.uint32(1), jnp.uint32(0))
        z = zi if z is None else z | zi
    z = jnp.concatenate([z] * (lhs_u32.shape[1] // 128), axis=1)
    if lhs_u32.shape[0] == 8:
        return lhs_u32 | z
    return jnp.concatenate([lhs_u32[0:8, :] | z, lhs_u32[8:, :]], axis=0)


def _gate_f(lhs, dep):
    z = _zero_f(dep)
    return lhs + jnp.concatenate([z] * (lhs.shape[1] // 128), axis=1)


def _run(main, streams=(), hooks=None):
    hooks = hooks or {}
    at = {}
    for tasks, first, last, lag in streams:
        n = len(tasks)
        for t, task in enumerate(tasks):
            at.setdefault(first + t * (last - first) // n, []).append((task, lag if t < n - 1 else lag + 2))
    pending = {}
    for i, m in enumerate(main):
        tok = m(pending.pop(i, []))
        for task, lag in at.get(i, []):
            o = task(tok)
            if o is not None:
                pending.setdefault(i + lag, []).append(o)
        for h in hooks.get(i, []):
            h()


def _kernel(x_hbm, lre_hbm, lim_hbm, ldt_hbm, dsk_hbm, wr_hbm, bre_hbm, bim_hbm, cre_hbm, cim_hbm,
            wg_hbm, wu_hbm, wd_hbm, out_hbm,
            x_v, xn_v, b_v, cre_v, cim_v, wg_v, wu_v, wd_v, out_v, sm_v, act_v, xb_v, *rest):
    S = rest[0:N]
    H = rest[N:2 * N]
    sem, sem_f = rest[2 * N:]
    SEM_S, SEM_X0, SEM_X1, SEM_B0, SEM_C, SEM_W, SEM_D, SEM_O = 0, 1, 2, 3, 8, 9, 10, 11

    def cp_x(j):
        return pltpu.make_async_copy(x_hbm.at[j * T:(j + 1) * T, :], x_v.at[j * T:(j + 1) * T, :],
                                     sem.at[(SEM_X0, SEM_X1, SEM_B0 + 4)[j] if j < 3 else SEM_C])

    def cp_b(p):
        k0, k1 = B_PIECES[p]
        return [pltpu.make_async_copy(src.at[k0:k1], b_v.at[k0:k1, c], sem.at[SEM_B0 + p])
                for c, src in enumerate((bre_hbm, bim_hbm))]

    cp_c = [pltpu.make_async_copy(cre_hbm, cre_v, sem.at[SEM_C]), pltpu.make_async_copy(cim_hbm, cim_v, sem.at[SEM_C])]
    cp_w = [pltpu.make_async_copy(wg_hbm, wg_v, sem.at[SEM_W]), pltpu.make_async_copy(wu_hbm, wu_v, sem.at[SEM_W]),
            pltpu.make_async_copy(wd_hbm, wd_v, sem.at[SEM_D])]
    cp_s = [pltpu.make_async_copy(h, sm_v.at[i], sem.at[SEM_S])
            for i, h in enumerate((lre_hbm, lim_hbm, ldt_hbm, dsk_hbm, wr_hbm))]

    def cp_o(j):
        return pltpu.make_async_copy(out_v.at[j * T:(j + 1) * T, :], out_hbm.at[j * T:(j + 1) * T, :], sem.at[SEM_O])

    order = ([cp_x(0)] + cp_s + cp_b(0) + [cp_x(1)] + cp_b(1) + cp_b(2) + cp_b(3) + [cp_x(2)] + cp_b(4) + cp_c
             + [cp_x(jj) for jj in range(3, N)] + cp_w)
    for c in order:
        c.start()
        pl.semaphore_signal(sem_f, 1)
        pl.semaphore_wait(sem_f, 1)

    cp_x(0).wait()
    for c in cp_s:
        c.wait()
    lre = sm_v[0].astype(f32)
    lim = sm_v[1].astype(f32)
    dt = _rb(jnp.exp(sm_v[2].astype(f32)))
    mag = jnp.exp(dt * lre)
    ang = dt * lim
    ar = mag * jnp.cos(ang)
    ai = mag * jnp.sin(ang)
    nr = ar - 1.0
    inv = 2.0 / (lre * lre + lim * lim)
    fr = (nr * lre + ai * lim) * inv
    fi = (ai * lre - nr * lim) * inv
    dsk1 = _row(sm_v[3].astype(f32)) + 1.0
    wr = _row(sm_v[4].astype(f32))

    def x_f32(r0, tok):
        xa = x_v[r0:r0 + 8, :].astype(f32)
        if tok is not None:
            xa = jnp.concatenate([xa[:, 0:128] + _zero_f(tok), xa[:, 128:]], axis=1)
        return jnp.concatenate([xa, x_v[r0 + 8:r0 + 16, :].astype(f32)], axis=0)

    def ln_group(r0, fast, tok):
        x = x_f32(r0, tok)
        mu = jnp.sum(x, axis=-1, keepdims=True) * (1.0 / D)
        mb = _rb(mu)
        xc = x - mb
        ex2 = jnp.sum(xc * xc, axis=-1, keepdims=True) * (1.0 / D)
        dm = mu - mb
        var = jnp.maximum(ex2 - dm * dm, 0.0)
        den = _rb(jnp.sqrt(_rb(_rb(var) + EPS_BF16)))
        xn = xc * (1.0 / den)
        xn_v[r0 // 2:(r0 + LNG) // 2, :] = pltpu.bitcast(xn.astype(bf16), u32)
        if fast:
            return None
        return r_part(r0, xn)

    racc = {"v": jnp.zeros((LNG, 128), f32)}
    lane_iota = lax.broadcasted_iota(jnp.int32, (LNG, 128), 1)

    def r_part(r0, xn):
        xw = xn * wr
        ps = xw[:, 0:128]
        for c in range(1, 8):
            ps = ps + xw[:, c * 128:(c + 1) * 128]
        r = _rb(jnp.sum(ps, axis=-1, keepdims=True))
        racc["v"] = jnp.where(lane_iota == r0 // LNG, r, racc["v"])
        return ps[0:8, :] + ps[8:16, :]

    def ln_fast(j):
        for g in range(T // LNG):
            ln_group(j * T + g * LNG, True, None)

    def ln_tasks(j):
        return [(lambda tok, r0=j * T + g * LNG: ln_group(r0, False, tok)) for g in range(T // LNG)]

    def rest_group(r0, tok):
        xu = xn_v[r0 // 2:(r0 + LNG) // 2, :]
        xn = pltpu.bitcast(_gate(xu, [tok]), bf16).astype(f32)
        return r_part(r0, xn)

    def rest_tasks(j):
        return [(lambda tok, r0=j * T + g * LNG: rest_group(r0, tok)) for g in range(T // LNG)]

    def xn_u32(r0, r1, c0, c1):
        return xn_v[r0 // 2:r1 // 2, c0:c1]

    def s_store(j, k, re, im):
        frk = fr[k:k + 1, :]
        fik = fi[k:k + 1, :]
        S[j][pl.ds(k * TS, T, stride=2), :] = frk * re - fik * im
        S[j][pl.ds(k * TS + 1, T, stride=2), :] = frk * im + fik * re

    def mm1_units(j, nchunk=1, k0=0, k1=8):
        acc = {}

        def unit(k, c, h):
            def run(deps):
                lhs = _gate(xn_u32(j * T, (j + nchunk) * T, h * KU, (h + 1) * KU), deps)
                part = _dot(pltpu.bitcast(lhs, bf16), b_v[k, c, :, h * KU:(h + 1) * KU], NT)
                acc[(k, c)] = part if h == 0 else acc[(k, c)] + part
                if c == 1 and h == 1:
                    re = acc.pop((k, 0))
                    im = acc.pop((k, 1))
                    for cc in range(nchunk):
                        s_store(j + cc, k, re[cc * T:(cc + 1) * T], im[cc * T:(cc + 1) * T])
                return part[0:8, :]
            return run
        return [unit(k, c, h) for k in range(k0, k1) for c in range(2) for h in range(D // KU)]

    hst = {"r": jnp.zeros((8, 128), f32), "i": jnp.zeros((8, 128), f32)}

    def scan_seg(j, t0, t1, tok):
        s = S[j]
        h = H[j]
        hr, hi = hst["r"], hst["i"]
        if tok is not None:
            hr = hr + _zero_f(tok)
        for t2 in range(t0 // 2, t1 // 2):
            outs = []
            for t in (2 * t2, 2 * t2 + 1):
                ur = s[pl.ds(2 * t, 8, stride=TS), :]
                ui = s[pl.ds(2 * t + 1, 8, stride=TS), :]
                nr_ = ar * hr - ai * hi + ur
                ni_ = ar * hi + ai * hr + ui
                hr, hi = nr_, ni_
                outs.append((hr, hi))
            h[pl.ds(2 * t2, 8, stride=TH), :] = _pack2(outs[0][0], outs[1][0])
            h[pl.ds(2 * t2 + 1, 8, stride=TH), :] = _pack2(outs[0][1], outs[1][1])
        hst["r"], hst["i"] = hr, hi
        return hr

    def scan_tasks(j, nseg=SCAN_SEGS):
        w = T // nseg
        return [(lambda tok, a=a: scan_seg(j, a, a + w, tok)) for a in range(0, T, w)]

    def h_u32(j, k):
        return H[j][pl.ds((k % 8) * TH + k // 8, T // 2, stride=2), :]

    def mm2_units(j):
        rows = slice(j * T, (j + 1) * T)
        acc = {}

        def unit(q, u):
            def run(deps):
                cols = slice(q * 128, (q + 1) * 128)
                ks = slice((u % 2) * KU, (u % 2 + 1) * KU)
                lhs = jnp.concatenate([h_u32(j, 4 * u + a) for a in range(4)], axis=1)
                lhs = pltpu.bitcast(_gate(lhs, deps), bf16)
                cw = cre_v if u < 2 else cim_v
                part = _dot(lhs, cw[cols, ks], NT)
                if u == 0:
                    acc[q] = part
                elif u == 1:
                    acc[q] = acc[q] + part
                elif u == 2:
                    acc[q] = acc[q] - part
                else:
                    xq = x_v[rows, cols].astype(f32)
                    xnq = pltpu.bitcast(xn_v[j * T // 2:(j + 1) * T // 2, cols], bf16).astype(f32)
                    o = (acc.pop(q) - part) + (xq + xnq * dsk1[:, cols])
                    if j >= NPATCH:
                        rid = lax.broadcasted_iota(jnp.int32, (T, 128), 0) + j * T
                        for k, i in enumerate(st["i"]):
                            o = o + jnp.where(rid == i, st["upd"][k:k + 1, cols], 0.0)
                    out_v[rows, cols] = o
                return part[0:8, :]
            return run
        return [unit(q, u) for q in range(8) for u in range(4)]

    st = {}

    def top2():
        vals = racc["v"]
        idxs = (lane_iota * LNG + lax.broadcasted_iota(jnp.int32, (LNG, 128), 0)).astype(f32)

        def amax(v):
            return jnp.max(jnp.max(v, axis=1, keepdims=True), axis=0, keepdims=True)

        def amin(v):
            return jnp.min(jnp.min(v, axis=1, keepdims=True), axis=0, keepdims=True)

        m1 = amax(vals)
        i1f = amin(jnp.where(vals == m1, idxs, float(L)))
        vals2 = jnp.where(idxs == i1f, -jnp.inf, vals)
        m2 = amax(vals2)
        i2f = amin(jnp.where(vals2 == m2, idxs, float(L)))
        i1 = jnp.clip(jnp.min(i1f).astype(jnp.int32), 0, L - 1)
        i2 = jnp.clip(jnp.min(i2f).astype(jnp.int32), 0, L - 1)

        def gather(i):
            base = pl.multiple_of((i // 16) * 8, 8)
            tile = pltpu.bitcast(xn_v[pl.ds(base, 8), :], bf16).astype(f32)
            sel = lax.broadcasted_iota(jnp.int32, (16, D), 0) == (i % 16)
            return jnp.sum(jnp.where(sel, tile, 0.0), axis=0, keepdims=True)

        for tok, i in enumerate((i1, i2)):
            row = gather(i)
            a = jnp.concatenate([row[:, c * 128:(c + 1) * 128] for c in range(8)], axis=0)
            at = a.T
            for c in range(8):
                for m in range(16):
                    g = tok * 128 + 16 * c + m
                    xb_v[8 * g:8 * g + 8, :] = jnp.broadcast_to(at[8 * m:8 * m + 8, c:c + 1], (8, 128))
        st["i"] = (i1, i2)
        st["m"] = (m1, m2)

    def gu_units():
        def unit(k, w, h):
            def run(dep):
                cols = slice(k * 128, (k + 1) * 128)
                key = ("gu", k, w)
                if h == 0:
                    a0 = _zero_f(dep)
                    a1 = jnp.zeros((8, 128), f32)
                else:
                    a0, a1 = st[key]
                    a0 = a0 + _zero_f(dep)
                wref = (wg_v, wu_v)[w]
                for g in range(h * 64, (h + 1) * 64):
                    wt = wref[8 * g:8 * g + 8, cols].astype(f32)
                    a0 = a0 + wt * xb_v[8 * g:8 * g + 8, :]
                    a1 = a1 + wt * xb_v[8 * (128 + g):8 * (128 + g) + 8, :]
                st[key] = (a0, a1)
                if w == 1 and h == 1:
                    g0, g1 = (jnp.sum(v, axis=0, keepdims=True) for v in st.pop(("gu", k, 0)))
                    u0, u1 = (jnp.sum(v, axis=0, keepdims=True) for v in st.pop(("gu", k, 1)))
                    rid = lax.broadcasted_iota(jnp.int32, (8, 128), 0)
                    gg = jnp.where(rid == 0, g0, jnp.where(rid == 1, g1, 0.0))
                    uu = jnp.where(rid == 0, u0, jnp.where(rid == 1, u1, 0.0))
                    act_v[:, cols] = _rb(gg * jax.nn.sigmoid(gg) * uu)
                return a0
            return run
        return [unit(k, w, h) for k in range(F // 128) for w in range(2) for h in range(2)]

    def down_units():
        def unit(q, u):
            def run(dep):
                cols = slice(q * 128, (q + 1) * 128)
                ks = slice(u * KU, (u + 1) * KU)
                lhs = _gate_f(act_v[:, ks], dep)
                part = _dot(lhs, wd_v[ks, cols].astype(f32), NN)
                key = ("y", q)
                st[key] = part if u == 0 else st[key] + part
                return part[0:8, :]
            return run
        return [unit(q, u) for q in range(8) for u in range(F // KU)]

    def patch():
        m1, m2 = st["m"]
        y = jnp.concatenate([st[("y", q)] for q in range(8)], axis=1)
        rid = lax.broadcasted_iota(jnp.int32, (8, D), 0)
        rs = jnp.where(rid == 0, m1, m2)
        st["upd"] = y * jax.nn.sigmoid(rs)
        for k, i in enumerate(st["i"]):
            g0 = pl.multiple_of(jnp.minimum(i // 8, NPATCH * T // 8 - 1) * 8, 8)
            sel = lax.broadcasted_iota(jnp.int32, (8, D), 0) == (i - g0)
            blk = out_v[pl.ds(g0, 8), :]
            out_v[pl.ds(g0, 8), :] = blk + jnp.where(sel, st["upd"][k:k + 1, :], 0.0)

    def wait_all(cs):
        for c in cs:
            c.wait()

    ln_fast(0)
    wait_all(cp_b(0))
    _run(mm1_units(0, 1, *B_PIECES[0]))
    cp_x(1).wait()
    ln_fast(1)
    _run(mm1_units(1, 1, *B_PIECES[0]))
    wait_all(cp_b(1))
    _run(mm1_units(0, 2, *B_PIECES[1]))
    wait_all(cp_b(2))
    _run(mm1_units(0, 2, *B_PIECES[2]))
    wait_all(cp_b(3))
    _run(mm1_units(0, 2, *B_PIECES[3]))
    wait_all(cp_b(4) + [cp_x(2)])
    _run(mm1_units(0, 2, *B_PIECES[4]) + mm1_units(2),
         [(ln_tasks(2), 0, 6, 2), (rest_tasks(0) + rest_tasks(1), 8, 24, 2), (scan_tasks(0), 10, 38, 2)])
    wait_all(cp_c + [cp_x(jj) for jj in range(3, N)])
    _run(mm2_units(0) + mm1_units(3) + mm2_units(1) + mm1_units(4),
         [(ln_tasks(3), 0, 20, 3), (scan_tasks(1), 0, 30, 2),
          (ln_tasks(4), 20, 40, 3), (scan_tasks(2), 32, 62, 2),
          (ln_tasks(5), 40, 60, 3),
          (ln_tasks(6), 60, 80, 3), (scan_tasks(3), 66, 94, 2),
          (ln_tasks(7), 80, 100, 3)],
         {106: [top2]})
    wait_all(cp_w[0:2])
    gu = gu_units()
    dn = down_units()
    _run(mm2_units(2) + mm1_units(5) + mm2_units(3),
         [(gu[0:96], 0, 94, GU_LAG), (scan_tasks(4), 0, 92, 2)])
    cp_w[2].wait()
    cp_l = [pltpu.make_async_copy(out_v.at[7 * T:8 * T, q * 128:(q + 1) * 128],
                                  out_hbm.at[7 * T:8 * T, q * 128:(q + 1) * 128], sem.at[SEM_O]) for q in range(8)]
    hooks = {82: [patch] + [cp_o(jj).start for jj in range(5)], 127: [cp_o(5).start], 159: [cp_o(6).start]}
    for q in range(8):
        hooks[160 + 4 * q + 3] = [cp_l[q].start]
    _run(mm1_units(6) + mm2_units(4) + mm1_units(7) + mm2_units(5) + mm2_units(6) + mm2_units(7),
         [(gu[96:112], 0, 16, GU_LAG), (dn, 21, 77, 2), (scan_tasks(5), 8, 34, 2), (scan_tasks(6), 36, 64, 2),
          (scan_tasks(7), 98, 126, 2)], hooks)
    pltpu.make_async_copy(out_v, out_hbm, sem.at[SEM_O]).wait()


@jax.jit
def pallas_parallel_sum__ssm_conv_s5__moe_arch_mod__prompt_kernel(A_x, A_Lambda_re, A_Lambda_im, A_B_re, A_B_im, A_C_re, A_C_im, A_log_dt, A_Dskip,
              B_x, B_w_r, B_w_gate, B_w_up, B_w_down):
    x = A_x.reshape(L, D)
    s8 = lambda v: v.reshape(8, 128)
    any_spec = pl.BlockSpec(memory_space=pl.ANY)
    out = pl.pallas_call(
        _kernel,
        out_shape=jax.ShapeDtypeStruct((L, D), f32),
        in_specs=[any_spec] * 13,
        out_specs=any_spec,
        scratch_shapes=[
            pltpu.VMEM((L, D), bf16),
            pltpu.VMEM((L // 2, D), u32),
            pltpu.VMEM((8, 2, 128, D), bf16),
            pltpu.VMEM((D, P), bf16),
            pltpu.VMEM((D, P), bf16),
            pltpu.VMEM((D, F), bf16),
            pltpu.VMEM((D, F), bf16),
            pltpu.VMEM((F, D), bf16),
            pltpu.VMEM((L, D), f32),
            pltpu.VMEM((5, 8, 128), bf16),
            pltpu.VMEM((8, F), f32),
            pltpu.VMEM((2 * 128 * 8, 128), f32),
        ] + [pltpu.VMEM((9 * TS, 128), f32) for _ in range(N)]
          + [pltpu.VMEM((9 * TH, 128), u32) for _ in range(N)] + [
            pltpu.SemaphoreType.DMA((12,)),
            pltpu.SemaphoreType.REGULAR,
        ],
        compiler_params=pltpu.CompilerParams(vmem_limit_bytes=110 * 1024 * 1024),
    )(x, s8(A_Lambda_re), s8(A_Lambda_im), s8(A_log_dt), s8(A_Dskip), s8(B_w_r),
      A_B_re.reshape(8, 128, D), A_B_im.reshape(8, 128, D), A_C_re, A_C_im, B_w_gate, B_w_up, B_w_down)
    return out.reshape(1, L, D)
```

```python
import jax
import jax.numpy as jnp
from jax import lax
import jax.experimental.pallas as pl
import jax.experimental.pallas.tpu as pltpu

L = 2048
D = 1024
P = 1024
F = 3584
T = 256
N = L // T
TS = 2 * T + 4
TH = T + 4
NT = (((1,), (1,)), ((), ()))
NN = (((1,), (0,)), ((), ()))
f32 = jnp.float32
bf16 = jnp.bfloat16
u32 = jnp.uint32
EPS_BF16 = 1.0013580322265625e-05
B_PIECES = ((0, 1), (1, 2), (2, 4), (4, 6), (6, 8))
LNG = 16
KU = 512
SCAN_SEGS = 16
NPATCH = 5
LN_LAG, SCAN_LAG, GU_LAG = 4, 2, 3


def _rb(v):
    return v.astype(bf16).astype(f32)


def _row(v8):
    return jnp.concatenate([v8[j:j + 1, :] for j in range(8)], axis=1)


def _dot(a, b, dims):
    return lax.dot_general(a, b, dims, preferred_element_type=f32)


def _zero_f(v):
    return jnp.where(v > jnp.inf, 1.0, 0.0)


def _pack2(a, b):
    ua = lax.bitcast_convert_type(a, u32) + jnp.uint32(0x8000)
    ub = lax.bitcast_convert_type(b, u32) + jnp.uint32(0x8000)
    return (ua >> 16) | (ub & jnp.uint32(0xFFFF0000))


def _gate(lhs_u32, deps):
    if not deps:
        return lhs_u32
    z = None
    for d in deps:
        zi = jnp.where(d > jnp.inf, jnp.uint32(1), jnp.uint32(0))
        z = zi if z is None else z | zi
    z = jnp.concatenate([z] * (lhs_u32.shape[1] // 128), axis=1)
    if lhs_u32.shape[0] == 8:
        return lhs_u32 | z
    return jnp.concatenate([lhs_u32[0:8, :] | z, lhs_u32[8:, :]], axis=0)


def _run(main, streams=(), hooks=None):
    hooks = hooks or {}
    at = {}
    for tasks, first, last, lag in streams:
        n = len(tasks)
        for t, task in enumerate(tasks):
            at.setdefault(first + t * (last - first) // n, []).append((task, lag if t < n - 1 else lag + 2))
    pending = {}
    for i, m in enumerate(main):
        tok = m(pending.pop(i, []))
        for task, lag in at.get(i, []):
            pending.setdefault(i + lag, []).append(task(tok))
        for h in hooks.get(i, []):
            h()


def _kernel(x_hbm, lre_hbm, lim_hbm, ldt_hbm, dsk_hbm, wr_hbm, bre_hbm, bim_hbm, cre_hbm, cim_hbm,
            wg_hbm, wu_hbm, wd_hbm, out_hbm,
            x_v, xn_v, b_v, cre_v, cim_v, wg_v, wu_v, wd_v, out_v, sm_v, act_v, xb_v, *rest):
    S = rest[0:N]
    H = rest[N:2 * N]
    sem, sem_f = rest[2 * N:]
    SEM_S, SEM_X0, SEM_X1, SEM_B0, SEM_C, SEM_W, SEM_D, SEM_O = 0, 1, 2, 3, 8, 9, 10, 11

    def cp_x(j):
        return pltpu.make_async_copy(x_hbm.at[j * T:(j + 1) * T, :], x_v.at[j * T:(j + 1) * T, :],
                                     sem.at[(SEM_X0, SEM_X1, SEM_B0 + 4)[j] if j < 3 else SEM_C])

    def cp_b(p):
        k0, k1 = B_PIECES[p]
        return [pltpu.make_async_copy(src.at[k0:k1], b_v.at[k0:k1, c], sem.at[SEM_B0 + p])
                for c, src in enumerate((bre_hbm, bim_hbm))]

    cp_c = [pltpu.make_async_copy(cre_hbm, cre_v, sem.at[SEM_C]), pltpu.make_async_copy(cim_hbm, cim_v, sem.at[SEM_C])]
    cp_w = [pltpu.make_async_copy(wg_hbm, wg_v, sem.at[SEM_W]), pltpu.make_async_copy(wu_hbm, wu_v, sem.at[SEM_W]),
            pltpu.make_async_copy(wd_hbm, wd_v, sem.at[SEM_D])]
    cp_s = [pltpu.make_async_copy(h, sm_v.at[i], sem.at[SEM_S])
            for i, h in enumerate((lre_hbm, lim_hbm, ldt_hbm, dsk_hbm, wr_hbm))]

    def cp_o(j):
        return pltpu.make_async_copy(out_v.at[j * T:(j + 1) * T, :], out_hbm.at[j * T:(j + 1) * T, :], sem.at[SEM_O])

    def cp_last(q):
        cols = slice(q * 128, (q + 1) * 128)
        return pltpu.make_async_copy(out_v.at[(N - 1) * T:N * T, cols], out_hbm.at[(N - 1) * T:N * T, cols],
                                     sem.at[SEM_O])

    def wait_all(cs):
        for c in cs:
            c.wait()

    order = ([cp_x(0)] + cp_s + cp_b(0) + [cp_x(1)] + cp_b(1) + cp_b(2) + cp_b(3) + [cp_x(2)] + cp_b(4) + cp_c
             + [cp_x(jj) for jj in range(3, N)] + cp_w)
    for c in order:
        c.start()
        pl.semaphore_signal(sem_f, 1)
        pl.semaphore_wait(sem_f, 1)

    cp_x(0).wait()
    wait_all(cp_s)
    lre = sm_v[0].astype(f32)
    lim = sm_v[1].astype(f32)
    dt = _rb(jnp.exp(sm_v[2].astype(f32)))
    mag = jnp.exp(dt * lre)
    ang = dt * lim
    ar = mag * jnp.cos(ang)
    ai = mag * jnp.sin(ang)
    nr = ar - 1.0
    inv = 2.0 / (lre * lre + lim * lim)
    fr = (nr * lre + ai * lim) * inv
    fi = (ai * lre - nr * lim) * inv
    dsk1 = _row(sm_v[3].astype(f32)) + 1.0
    wr = _row(sm_v[4].astype(f32))

    lane_iota = lax.broadcasted_iota(jnp.int32, (LNG, 128), 1)
    st = {"racc": jnp.zeros((LNG, 128), f32),
          "hr": jnp.zeros((8, 128), f32), "hi": jnp.zeros((8, 128), f32)}

    def router(r0, xn):
        xw = xn * wr
        ps = xw[:, 0:128]
        for c in range(1, 8):
            ps = ps + xw[:, c * 128:(c + 1) * 128]
        r = _rb(jnp.sum(ps, axis=-1, keepdims=True))
        st["racc"] = jnp.where(lane_iota == r0 // LNG, r, st["racc"])
        return ps[0:8, :] + ps[8:16, :]

    def ln_group(r0, tok):
        xa = x_v[r0:r0 + 8, :].astype(f32)
        if tok is not None:
            xa = jnp.concatenate([xa[:, 0:128] + _zero_f(tok), xa[:, 128:]], axis=1)
        x = jnp.concatenate([xa, x_v[r0 + 8:r0 + 16, :].astype(f32)], axis=0)
        mu = jnp.sum(x, axis=-1, keepdims=True) * (1.0 / D)
        mb = _rb(mu)
        xc = x - mb
        ex2 = jnp.sum(xc * xc, axis=-1, keepdims=True) * (1.0 / D)
        dm = mu - mb
        var = jnp.maximum(ex2 - dm * dm, 0.0)
        den = _rb(jnp.sqrt(_rb(_rb(var) + EPS_BF16)))
        xn = xc * (1.0 / den)
        xn_v[r0 // 2:(r0 + LNG) // 2, :] = pltpu.bitcast(xn.astype(bf16), u32)
        return xn

    def ln_fast(j):
        for r0 in range(j * T, (j + 1) * T, LNG):
            ln_group(r0, None)

    def ln_tasks(j):
        return [(lambda tok, r0=r0: router(r0, ln_group(r0, tok))) for r0 in range(j * T, (j + 1) * T, LNG)]

    def router_group(r0, tok):
        xu = xn_v[r0 // 2:(r0 + LNG) // 2, :]
        return router(r0, pltpu.bitcast(_gate(xu, [tok]), bf16).astype(f32))

    def router_tasks(j):
        return [(lambda tok, r0=r0: router_group(r0, tok)) for r0 in range(j * T, (j + 1) * T, LNG)]

    def s_store(j, k, re, im):
        frk = fr[k:k + 1, :]
        fik = fi[k:k + 1, :]
        S[j][pl.ds(k * TS, T, stride=2), :] = frk * re - fik * im
        S[j][pl.ds(k * TS + 1, T, stride=2), :] = frk * im + fik * re

    def mm1_units(j, nchunk=1, k0=0, k1=8):
        acc = {}

        def unit(k, c, h):
            def run(deps):
                lhs = _gate(xn_v[j * T // 2:(j + nchunk) * T // 2, h * KU:(h + 1) * KU], deps)
                part = _dot(pltpu.bitcast(lhs, bf16), b_v[k, c, :, h * KU:(h + 1) * KU], NT)
                acc[(k, c)] = part if h == 0 else acc[(k, c)] + part
                if c == 1 and h == 1:
                    re = acc.pop((k, 0))
                    im = acc.pop((k, 1))
                    for cc in range(nchunk):
                        s_store(j + cc, k, re[cc * T:(cc + 1) * T], im[cc * T:(cc + 1) * T])
                return part[0:8, :]
            return run
        return [unit(k, c, h) for k in range(k0, k1) for c in range(2) for h in range(D // KU)]

    def scan_seg(j, t0, t1, tok):
        s = S[j]
        h = H[j]
        hr, hi = st["hr"] + _zero_f(tok), st["hi"]
        for t2 in range(t0 // 2, t1 // 2):
            outs = []
            for t in (2 * t2, 2 * t2 + 1):
                ur = s[pl.ds(2 * t, 8, stride=TS), :]
                ui = s[pl.ds(2 * t + 1, 8, stride=TS), :]
                hr, hi = ar * hr - ai * hi + ur, ar * hi + ai * hr + ui
                outs.append((hr, hi))
            h[pl.ds(2 * t2, 8, stride=TH), :] = _pack2(outs[0][0], outs[1][0])
            h[pl.ds(2 * t2 + 1, 8, stride=TH), :] = _pack2(outs[0][1], outs[1][1])
        st["hr"], st["hi"] = hr, hi
        return hr

    def scan_tasks(j):
        w = T // SCAN_SEGS
        return [(lambda tok, a=a: scan_seg(j, a, a + w, tok)) for a in range(0, T, w)]

    def mm2_units(j):
        rows = slice(j * T, (j + 1) * T)
        acc = {}

        def h_u32(k):
            return H[j][pl.ds((k % 8) * TH + k // 8, T // 2, stride=2), :]

        def unit(q, u):
            def run(deps):
                cols = slice(q * 128, (q + 1) * 128)
                ks = slice((u % 2) * KU, (u % 2 + 1) * KU)
                lhs = jnp.concatenate([h_u32(4 * u + a) for a in range(4)], axis=1)
                lhs = pltpu.bitcast(_gate(lhs, deps), bf16)
                cw = cre_v if u < 2 else cim_v
                part = _dot(lhs, cw[cols, ks], NT)
                if u == 0:
                    acc[q] = part
                elif u == 1:
                    acc[q] = acc[q] + part
                elif u == 2:
                    acc[q] = acc[q] - part
                else:
                    xq = x_v[rows, cols].astype(f32)
                    xnq = pltpu.bitcast(xn_v[j * T // 2:(j + 1) * T // 2, cols], bf16).astype(f32)
                    o = (acc.pop(q) - part) + (xq + xnq * dsk1[:, cols])
                    if j >= NPATCH:
                        rid = lax.broadcasted_iota(jnp.int32, (T, 128), 0) + j * T
                        for k, i in enumerate(st["i"]):
                            o = o + jnp.where(rid == i, st["upd"][k:k + 1, cols], 0.0)
                    out_v[rows, cols] = o
                return part[0:8, :]
            return run
        return [unit(q, u) for q in range(8) for u in range(4)]

    def top2():
        vals = st["racc"]
        idxs = (lane_iota * LNG + lax.broadcasted_iota(jnp.int32, (LNG, 128), 0)).astype(f32)

        def amax(v):
            return jnp.max(jnp.max(v, axis=1, keepdims=True), axis=0, keepdims=True)

        def amin(v):
            return jnp.min(jnp.min(v, axis=1, keepdims=True), axis=0, keepdims=True)

        m1 = amax(vals)
        i1f = amin(jnp.where(vals == m1, idxs, float(L)))
        vals2 = jnp.where(idxs == i1f, -jnp.inf, vals)
        m2 = amax(vals2)
        i2f = amin(jnp.where(vals2 == m2, idxs, float(L)))
        i1 = jnp.clip(jnp.min(i1f).astype(jnp.int32), 0, L - 1)
        i2 = jnp.clip(jnp.min(i2f).astype(jnp.int32), 0, L - 1)

        def gather(i):
            base = pl.multiple_of((i // 16) * 8, 8)
            tile = pltpu.bitcast(xn_v[pl.ds(base, 8), :], bf16).astype(f32)
            sel = lax.broadcasted_iota(jnp.int32, (16, D), 0) == (i % 16)
            return jnp.sum(jnp.where(sel, tile, 0.0), axis=0, keepdims=True)

        for tok, i in enumerate((i1, i2)):
            row = gather(i)
            at = jnp.concatenate([row[:, c * 128:(c + 1) * 128] for c in range(8)], axis=0).T
            for c in range(8):
                xb_v[tok * D + c * 128:tok * D + (c + 1) * 128, :] = jnp.broadcast_to(at[:, c:c + 1], (128, 128))
        st["i"] = (i1, i2)
        st["m"] = (m1, m2)

    def gu_tasks():
        def task(k, w, h):
            def run(dep):
                cols = slice(k * 128, (k + 1) * 128)
                key = ("gu", k, w)
                if h == 0:
                    a0 = _zero_f(dep)
                    a1 = jnp.zeros((8, 128), f32)
                else:
                    a0, a1 = st[key]
                    a0 = a0 + _zero_f(dep)
                wt = (wg_v, wu_v)[w][h * KU:(h + 1) * KU, cols].astype(f32)
                a0 = a0 + jnp.sum((wt * xb_v[h * KU:(h + 1) * KU, :]).reshape(KU // 8, 8, 128), axis=0)
                a1 = a1 + jnp.sum((wt * xb_v[D + h * KU:D + (h + 1) * KU, :]).reshape(KU // 8, 8, 128), axis=0)
                st[key] = (a0, a1)
                if w == 1 and h == 1:
                    g0, g1 = (jnp.sum(v, axis=0, keepdims=True) for v in st.pop(("gu", k, 0)))
                    u0, u1 = (jnp.sum(v, axis=0, keepdims=True) for v in st.pop(("gu", k, 1)))
                    rid = lax.broadcasted_iota(jnp.int32, (8, 128), 0)
                    gg = jnp.where(rid == 0, g0, jnp.where(rid == 1, g1, 0.0))
                    uu = jnp.where(rid == 0, u0, jnp.where(rid == 1, u1, 0.0))
                    act_v[:, cols] = _rb(gg * jax.nn.sigmoid(gg) * uu)
                return a0
            return run
        return [task(k, w, h) for k in range(F // 128) for w in range(2) for h in range(2)]

    def down_tasks():
        def task(q, u):
            def run(dep):
                cols = slice(q * 128, (q + 1) * 128)
                ks = slice(u * KU, (u + 1) * KU)
                lhs = act_v[:, ks] + jnp.concatenate([_zero_f(dep)] * (KU // 128), axis=1)
                part = _dot(lhs, wd_v[ks, cols].astype(f32), NN)
                key = ("y", q)
                st[key] = part if u == 0 else st[key] + part
                return part
            return run
        return [task(q, u) for q in range(8) for u in range(F // KU)]

    def patch():
        m1, m2 = st["m"]
        y = jnp.concatenate([st[("y", q)] for q in range(8)], axis=1)
        rid = lax.broadcasted_iota(jnp.int32, (8, D), 0)
        st["upd"] = y * jax.nn.sigmoid(jnp.where(rid == 0, m1, m2))
        for k, i in enumerate(st["i"]):
            g0 = pl.multiple_of(jnp.minimum(i // 8, NPATCH * T // 8 - 1) * 8, 8)
            sel = lax.broadcasted_iota(jnp.int32, (8, D), 0) == (i - g0)
            blk = out_v[pl.ds(g0, 8), :]
            out_v[pl.ds(g0, 8), :] = blk + jnp.where(sel, st["upd"][k:k + 1, :], 0.0)

    ln_fast(0)
    wait_all(cp_b(0))
    _run(mm1_units(0, 1, *B_PIECES[0]))
    cp_x(1).wait()
    ln_fast(1)
    _run(mm1_units(1, 1, *B_PIECES[0]))
    for p in range(1, 4):
        wait_all(cp_b(p))
        _run(mm1_units(0, 2, *B_PIECES[p]), [(router_tasks(p - 2), 0, 6, 2)] if p > 1 else [])
    wait_all(cp_b(4) + [cp_x(2)])
    _run(mm1_units(0, 2, *B_PIECES[4]) + mm1_units(2),
         [(ln_tasks(2), 0, 6, 2), (scan_tasks(0), 10, 38, SCAN_LAG)])
    wait_all(cp_c + [cp_x(jj) for jj in range(3, N)])
    _run(mm2_units(0) + mm1_units(3) + mm2_units(1) + mm1_units(4),
         [(ln_tasks(3), 0, 20, LN_LAG), (scan_tasks(1), 0, 30, SCAN_LAG),
          (ln_tasks(4), 20, 40, LN_LAG), (scan_tasks(2), 32, 62, SCAN_LAG),
          (ln_tasks(5), 40, 60, LN_LAG),
          (ln_tasks(6), 60, 80, LN_LAG), (scan_tasks(3), 66, 94, SCAN_LAG),
          (ln_tasks(7), 80, 100, LN_LAG)],
         {106: [top2]})
    wait_all(cp_w[0:2])
    gu = gu_tasks()
    _run(mm2_units(2) + mm1_units(5) + mm2_units(3),
         [(gu[0:96], 0, 94, GU_LAG), (scan_tasks(4), 0, 92, SCAN_LAG)])
    cp_w[2].wait()
    hooks = {82: [patch] + [cp_o(jj).start for jj in range(NPATCH)], 127: [cp_o(5).start], 159: [cp_o(6).start]}
    for q in range(8):
        hooks[160 + 4 * q + 3] = [cp_last(q).start]
    _run(mm1_units(6) + mm2_units(4) + mm1_units(7) + mm2_units(5) + mm2_units(6) + mm2_units(7),
         [(gu[96:112], 0, 16, GU_LAG), (down_tasks(), 21, 77, 2), (scan_tasks(5), 8, 34, SCAN_LAG),
          (scan_tasks(6), 36, 64, SCAN_LAG), (scan_tasks(7), 98, 126, SCAN_LAG)], hooks)
    pltpu.make_async_copy(out_v, out_hbm, sem.at[SEM_O]).wait()


@jax.jit
def pallas_parallel_sum__ssm_conv_s5__moe_arch_mod__prompt_kernel(
    A_x: jax.Array,
    A_Lambda_re: jax.Array,
    A_Lambda_im: jax.Array,
    A_B_re: jax.Array,
    A_B_im: jax.Array,
    A_C_re: jax.Array,
    A_C_im: jax.Array,
    A_log_dt: jax.Array,
    A_Dskip: jax.Array,
    B_x: jax.Array,
    B_w_r: jax.Array,
    B_w_gate: jax.Array,
    B_w_up: jax.Array,
    B_w_down: jax.Array,
):
    del B_x
    any_spec = pl.BlockSpec(memory_space=pl.ANY)
    out = pl.pallas_call(
        _kernel,
        out_shape=jax.ShapeDtypeStruct((L, D), f32),
        in_specs=[any_spec] * 13,
        out_specs=any_spec,
        scratch_shapes=[
            pltpu.VMEM((L, D), bf16),
            pltpu.VMEM((L // 2, D), u32),
            pltpu.VMEM((8, 2, 128, D), bf16),
            pltpu.VMEM((D, P), bf16),
            pltpu.VMEM((D, P), bf16),
            pltpu.VMEM((D, F), bf16),
            pltpu.VMEM((D, F), bf16),
            pltpu.VMEM((F, D), bf16),
            pltpu.VMEM((L, D), f32),
            pltpu.VMEM((5, 8, 128), bf16),
            pltpu.VMEM((8, F), f32),
            pltpu.VMEM((2 * D, 128), f32),
        ] + [pltpu.VMEM((9 * TS, 128), f32) for _ in range(N)]
          + [pltpu.VMEM((9 * TH, 128), u32) for _ in range(N)] + [
            pltpu.SemaphoreType.DMA((12,)),
            pltpu.SemaphoreType.REGULAR,
        ],
        compiler_params=pltpu.CompilerParams(vmem_limit_bytes=110 * 1024 * 1024),
    )(A_x.reshape(L, D), A_Lambda_re.reshape(8, 128), A_Lambda_im.reshape(8, 128), A_log_dt.reshape(8, 128),
      A_Dskip.reshape(8, 128), B_w_r.reshape(8, 128), A_B_re.reshape(8, 128, D), A_B_im.reshape(8, 128, D),
      A_C_re, A_C_im, B_w_gate, B_w_up, B_w_down)
    return out.reshape(1, L, D)
```
